```python
import jax
import jax.numpy as jnp

def _softmax(x, axis=-1):
    return jax.nn.softmax(x, axis=axis)
def _gelu(x):
    return jax.nn.gelu(x, approximate=True)
def _silu(x):
    return jax.nn.silu(x)
def _sigmoid(x):
    return jax.nn.sigmoid(x)
def _layernorm(x, axis=-1, eps=1e-5):
    m = jnp.mean(x, axis=axis, keepdims=True)
    v = jnp.var(x, axis=axis, keepdims=True)
    return (x - m) / jnp.sqrt(v + eps)
def _scatter_add(tgt, idx, src, axis=0):
    return tgt.at[idx].add(src)
def _segment_sum(src, seg, n):
    return jax.ops.segment_sum(src, seg, n)
class _Rng:
    def __init__(self, key):
        self._k = key
    def _next(self):
        self._k, sub = jax.random.split(self._k)
        return sub
    def normal(self, shape):
        return jax.random.normal(self._next(), shape, dtype=jnp.bfloat16)
    def randint(self, lo, hi, shape):
        return jax.random.randint(self._next(), shape, lo, hi, dtype=jnp.int32)
    def uniform(self, shape, lo=0.0, hi=1.0):
        return jax.random.uniform(self._next(), shape, jnp.bfloat16, lo, hi)
    def permutation(self, n):
        return jax.random.permutation(self._next(), n)


kernel_name = 'sequential_preLN__mha_block_cached__mixer_channel_mlp__decode'

def _fwd_setup_inputs():
    _rng = _Rng(jax.random.key(int.from_bytes(__import__("os").urandom(4), "little")))
    _w = (lambda a: (lambda t: t.astype(jnp.bfloat16) if jnp.issubdtype(t.dtype, jnp.floating) else t)(jnp.asarray(a)))
    def _A_setup():
        B, Sq, D = 2, 1, 512
        H, Sk, Dh = 32, 8192, 128
        return {
            "x": _w((lambda *s: _rng.normal(s) * 0.05)(B, Sq, D)),
            "k_cache": _w((lambda *s: _rng.normal(s) * 0.05)(B, H, Sk, Dh)),
            "v_cache": _w((lambda *s: _rng.normal(s) * 0.05)(B, H, Sk, Dh)),
            "wq": _w((lambda *s: _rng.normal(s) * 0.05)(D, H * Dh) * (D ** -0.5)),
            "wo": _w((lambda *s: _rng.normal(s) * 0.05)(H * Dh, D) * ((H * Dh) ** -0.5)),
        }
    _A_in = _A_setup()

    def _B_setup():
        B, S, D, F = 2, 1, 512, 1792
        return {
            "x": _w((lambda *s: _rng.normal(s) * 0.05)(B, S, D)),
            "w1": _w((lambda *s: _rng.normal(s) * 0.05)(D, F) * (D ** -0.5)),
            "b1": _w((lambda *s: _rng.normal(s) * 0.05)(F)),
            "w2": _w((lambda *s: _rng.normal(s) * 0.05)(F, D) * (F ** -0.5)),
            "b2": _w((lambda *s: _rng.normal(s) * 0.05)(D)),
        }
    _B_in = _B_setup()

    return {
        "A_x": _A_in["x"],
        "A_k_cache": _A_in["k_cache"],
        "A_v_cache": _A_in["v_cache"],
        "A_wq": _A_in["wq"],
        "A_wo": _A_in["wo"],
        "B_x": _B_in["x"],
        "B_w1": _B_in["w1"],
        "B_b1": _B_in["b1"],
        "B_w2": _B_in["w2"],
        "B_b2": _B_in["b2"],
    }

def _fwd_reference(A_x, A_k_cache, A_v_cache, A_wq, A_wo, B_x, B_w1, B_b1, B_w2, B_b2):
    def _A_ref(x, k_cache, v_cache, wq, wo):
        B, Sq, D = x.shape
        H, Dh = 32, 128
        q = (lambda x, *d: x.transpose(*d))((x @ wq).reshape(B, Sq, H, Dh), 0, 2, 1, 3)
        scores = jnp.einsum("bhqd,bhkd->bhqk", q, k_cache) * (Dh ** -0.5)
        p = _softmax(scores, axis=-1)
        o = jnp.einsum("bhqk,bhkd->bhqd", p, v_cache)
        return (lambda x, *d: x.transpose(*d))(o, 0, 2, 1, 3).reshape(B, Sq, H * Dh) @ wo

    def _B_ref(x, w1, b1, w2, b2):
        y = _layernorm(x, axis=-1)
        h = _gelu(jnp.einsum("bsd,df->bsf", y, w1) + b1)
        return jnp.einsum("bsf,fd->bsd", h, w2) + b2

    x = A_x
    h = x + _A_ref(_layernorm(x, axis=-1), A_k_cache, A_v_cache, A_wq, A_wo)
    h2 = h + _B_ref(_layernorm(h, axis=-1), B_w1, B_b1, B_w2, B_b2)
    return h2


def setup_inputs():
    _inp = _fwd_setup_inputs()
    _gk = jax.random.fold_in(jax.random.key(int.from_bytes(__import__("os").urandom(4), "little")), 2**31 - 1)
    _shapes = [[2, 1, 512]]
    _dtypes = ['bfloat16']
    _gks = jax.random.split(_gk, len(_shapes))
    _gs = [jax.random.normal(k, s, dtype=jnp.dtype(d)) * 0.05 for k, s, d in zip(_gks, _shapes, _dtypes)]
    _inp["grad_out"] = _gs[0]
    return _inp

def reference(A_x, A_k_cache, A_v_cache, A_wq, A_wo, B_w1, B_b1, B_w2, B_b2, B_x, grad_out):
    _const = dict(B_x=B_x)
    def _f(*_d):
        return _fwd_reference(**{'A_x': _d[0], 'A_k_cache': _d[1], 'A_v_cache': _d[2], 'A_wq': _d[3], 'A_wo': _d[4], 'B_w1': _d[5], 'B_b1': _d[6], 'B_w2': _d[7], 'B_b2': _d[8], **_const})
    _out, _vjp = jax.vjp(_f, A_x, A_k_cache, A_v_cache, A_wq, A_wo, B_w1, B_b1, B_w2, B_b2)
    _grads = _vjp(grad_out)
    _out0 = jnp.asarray(_out)
    return (_out0, *[jnp.asarray(_g) for _g in _grads])
```

```python
import jax
import jax.numpy as jnp
from jax import lax
import jax.experimental.pallas as pl
import jax.experimental.pallas.tpu as pltpu

BF = jnp.bfloat16
F32 = jnp.float32

B, H, S, DH, D, F = 2, 32, 8192, 128, 512, 1792
SCALE = DH ** -0.5
EPS = 1e-5

NK = 3
PF = 2
NV = H + PF
G = 8
NG = H // G
R = 512
C = 64
NN_ = S // R
SPB = 2 * NG * NN_
NS = 12
NDEF = 8
CH = 2048

NT = (((1,), (1,)), ((), ()))
NN = (((1,), (0,)), ((), ()))
TN = (((0,), (0,)), ((), ()))


def _dot(a, b, dims):
    return lax.dot_general(a, b, dims, preferred_element_type=F32)


def _ln_fwd(x):
    m = jnp.mean(x, axis=-1, keepdims=True)
    xc = x - m
    v = jnp.mean(xc * xc, axis=-1, keepdims=True)
    rstd = lax.rsqrt(v + EPS)
    return xc * rstd, rstd


def _ln_bwd(dy, y, rstd):
    m1 = jnp.mean(dy, axis=-1, keepdims=True)
    m2 = jnp.mean(dy * y, axis=-1, keepdims=True)
    return (dy - m1 - y * m2) * rstd


def _rows8(x2):
    return jnp.concatenate([x2.astype(F32), jnp.zeros((6, x2.shape[1]), F32)], axis=0)


def _kernel(x_hbm, k_hbm, v_hbm, wq_hbm, wo_hbm, w1_hbm, b1_hbm, w2_hbm, b2_hbm, g_hbm,
            out_hbm, dx_hbm, dk_hbm, dv_hbm, dwq_hbm, dwo_hbm, dw1_hbm, db1_hbm, dw2_hbm, db2_hbm,
            kbuf, vbuf, stage, wq_v, wo_v, w1_v, w2_v, x_v, g_v, b1_v, b2_v,
            coef, vec, o_s, hv, dq_s, mhi, mlo, s_s,
            xn_s, dh_s, y2_s, du_s, hid_s,
            out_v, dx_v, db1_v, db2_v,
            ksem, vsem, wsem, msem):

    def k_copy(t):
        return pltpu.make_async_copy(k_hbm.at[t // H, t % H], kbuf.at[t % NK], ksem.at[t % NK])

    def v_copy(t):
        return pltpu.make_async_copy(v_hbm.at[t // H, t % H], vbuf.at[t % NV], vsem.at[t % NK])

    def misc(src, dst, i):
        return pltpu.make_async_copy(src, dst, msem.at[i])

    def step_ids(j):
        r = j % SPB
        return j // SPB, r // (2 * NN_), (r // NN_) % 2, r % NN_

    def issue_step(j):
        b, g, kind, n = step_ids(j)
        slot = j % NS

        def issue(dst):
            for c in range(R // C):
                row = pl.multiple_of(n * R + c * C, C)
                pltpu.make_async_copy(
                    stage.at[slot, c],
                    dst.at[b, pl.ds(g * G, G), pl.ds(row, C)],
                    wsem.at[slot]).start()

        pl.when(kind == 0)(lambda: issue(dv_hbm))
        pl.when(kind == 1)(lambda: issue(dk_hbm))

    def wait_slot(slot):
        pltpu.make_async_copy(stage.at[slot], stage.at[slot], wsem.at[slot]).wait()

    in_small = [misc(x_hbm, x_v, 0), misc(g_hbm, g_v, 1), misc(b1_hbm, b1_v, 2), misc(b2_hbm, b2_v, 3)]
    in_wq = misc(wq_hbm, wq_v, 4)
    in_w = [misc(wo_hbm, wo_v, 5), misc(w1_hbm, w1_v, 6), misc(w2_hbm, w2_v, 7)]
    in_wq.start()
    for cp in in_small:
        cp.start()
    for t in range(PF):
        k_copy(t).start()
        v_copy(t).start()
    for cp in in_w:
        cp.start()

    o_s[...] = jnp.zeros(o_s.shape, F32)
    dq_s[...] = jnp.zeros(dq_s.shape, F32)

    for cp in in_small:
        cp.wait()
    xn, _ = _ln_fwd(_rows8(x_v[...]))
    xn_s[...] = xn
    in_wq.wait()
    q_all = _dot(xn.astype(BF), wq_v[...], NN).astype(BF).astype(F32)
    for bb in range(B):
        for h in range(H):
            vec[1, bb, h // G, pl.ds(h % G, 1), :] = q_all[bb:bb + 1, h * DH:(h + 1) * DH]

    row8 = lax.broadcasted_iota(jnp.int32, (8, DH), 0)

    def fwd_head(h, b):
        t = b * H + h
        g, i = h // G, h % G
        ks, vs = t % NK, t % NV
        col = pl.multiple_of(h * DH, DH)

        @pl.when(t + PF < B * H)
        def _():
            k_copy(t + PF).start()
            v_copy(t + PF).start()

        k_copy(t).wait()
        q8 = jnp.broadcast_to(vec[1, b, g, pl.ds(i, 1), :], (8, DH)).astype(BF)
        s_s[...] = _dot(q8, kbuf[ks], NT)
        s = s_s[...]
        m = jnp.max(s, axis=1, keepdims=True)
        e = jnp.exp((s - m) * SCALE)
        p = e * (1.0 / jnp.sum(e, axis=1, keepdims=True))
        s_s[...] = p
        coef[0, b, g, pl.ds(i, 1), :] = p[0:1, :]

        v_copy(t).wait()

        @pl.when(t == B * H - 1)
        def _():
            def issue_deferred(j, c):
                issue_step(j)
                return c
            lax.fori_loop(SPB - NDEF, SPB, issue_deferred, 0)

        def chunk(c, carry):
            acc, kb = carry
            r = pl.multiple_of(c * CH, CH)
            kc = kbuf[ks, pl.ds(r, CH), :]
            p8 = s_s[:, pl.ds(r, CH)]
            p_hi = p8.astype(BF)
            p_lo = (p8 - p_hi.astype(F32)).astype(BF)
            p16 = jnp.concatenate([p_hi, p_lo], axis=0)
            a = (kc.astype(F32).T * s_s[0:1, pl.ds(r, CH)]).astype(BF)
            acc = acc + _dot(jnp.concatenate([a, p16], axis=0), vbuf[vs, pl.ds(r, CH), :], NN)
            kb = kb + _dot(p16, kc, NN)
            return acc, kb

        acc, kb = lax.fori_loop(0, S // CH, chunk,
                                (jnp.zeros((DH + 16, DH), F32), jnp.zeros((16, DH), F32)))
        mt = acc[0:DH]
        mt_hi = mt.astype(BF)
        mhi[h] = mt_hi
        mlo[h] = (mt - mt_hi.astype(F32)).astype(BF)
        o8 = acc[DH:DH + 8] + acc[DH + 8:DH + 16]
        o_s[:, pl.ds(col, DH)] = jnp.where(row8 == b, o8, o_s[:, pl.ds(col, DH)])
        hv[0, g, pl.ds(i, 1), :] = o8[0:1]
        hv[1, g, pl.ds(i, 1), :] = kb[0:1] + kb[8:9]
        return b

    def middle(b):
        @pl.when(b == 0)
        def _():
            for cp in in_w:
                cp.wait()

        x8 = _rows8(x_v[...])
        g8 = _rows8(g_v[...])
        h1 = x8 + _dot(o_s[...].astype(BF), wo_v[...], NN)
        y1, r1 = _ln_fwd(h1)
        y2, r2 = _ln_fwd(y1)
        u = _dot(y2.astype(BF), w1_v[...], NN) + b1_v[...].astype(F32).reshape(1, F)
        c0 = (2.0 / jnp.pi) ** 0.5
        th = jnp.tanh(c0 * (u + 0.044715 * (u * u * u)))
        hid = 0.5 * u * (1.0 + th)
        dgelu = 0.5 * (1.0 + th) + 0.5 * u * (1.0 - th * th) * (c0 * (1.0 + 3 * 0.044715 * (u * u)))
        du = _dot(g8.astype(BF), w2_v[...], NT) * dgelu
        dy2 = _dot(du.astype(BF), w1_v[...], NT)
        dh = g8 + _ln_bwd(_ln_bwd(dy2, y2, r2), y1, r1)
        do_all = _dot(dh.astype(BF), wo_v[...], NT).astype(BF).astype(F32)
        row = lax.broadcasted_iota(jnp.int32, do_all.shape, 0)
        do_b = jnp.sum(jnp.where(row == b, do_all, 0.0), axis=0, keepdims=True)
        for h in range(H):
            vec[0, b, h // G, pl.ds(h % G, 1), :] = do_b[:, h * DH:(h + 1) * DH]
        dh_s[...] = dh
        y2_s[...] = y2
        du_s[...] = du
        hid_s[...] = hid
        out8 = h1 + _dot(hid.astype(BF), w2_v[...], NN) + b2_v[...].astype(F32).reshape(1, D)
        out_v[...] = out8[0:B].astype(BF)

    eye = (lax.broadcasted_iota(jnp.int32, (DH, DH), 0) == lax.broadcasted_iota(jnp.int32, (DH, DH), 1))

    def bwd_head(b, g, i):
        h = g * G + i
        col = pl.multiple_of(h * DH, DH)
        vs = (b * H + h) % NV
        do_row = vec[0, b, g, pl.ds(i, 1), :]
        dsum = jnp.sum(do_row * hv[0, g, pl.ds(i, 1), :], axis=1, keepdims=True)
        do8 = jnp.broadcast_to(do_row, (8, DH)).astype(BF)
        dq = _dot(do8, mhi[h], NT) + _dot(do8, mlo[h], NT)
        dq = (dq - dsum * hv[1, g, pl.ds(i, 1), :]) * SCALE
        dq_s[:, pl.ds(col, DH)] = jnp.where(row8 == b, dq, dq_s[:, pl.ds(col, DH)])
        dp = _dot(do8, vbuf[vs], NT)
        coef[1, b, g, pl.ds(i, 1), :] = coef[0, b, g, pl.ds(i, 1), :] * ((dp[0:1] - dsum) * SCALE)

    def w_step(j, carry):
        b, g, kind, n = step_ids(j)
        slot = j % NS
        drained = jnp.logical_and(j >= SPB, j < SPB + NS - NDEF - 1)

        @pl.when(jnp.logical_and(j >= NS, jnp.logical_not(drained)))
        def _():
            wait_slot(slot)

        for i in range(G):
            w = jnp.broadcast_to(vec[kind, b, g, pl.ds(i, 1), :], (DH, DH)).astype(BF)
            tiles = []
            for tt in range(R // DH):
                r = pl.multiple_of(n * R + tt * DH, DH)
                tiles.append(jnp.where(eye, coef[kind, b, g, pl.ds(i, 1), pl.ds(r, DH)], 0.0).astype(BF))
            res = _dot(jnp.concatenate(tiles, axis=0), w, NN).astype(BF)
            stage[slot, :, i] = res.reshape(R // C, C, DH)

        @pl.when(jnp.logical_or(j < SPB - NDEF, j >= SPB))
        def _():
            issue_step(j)

        @pl.when(jnp.logical_and(kind == 0, n % (NN_ // G) == NN_ // G - 1))
        def _():
            bwd_head(b, g, n // (NN_ // G))

        return carry

    def batch(b, carry):
        @pl.when(b == 1)
        def _():
            for j in range(SPB - NS, SPB - NDEF - 1):
                wait_slot(j % NS)

        lax.fori_loop(0, H, fwd_head, b)
        middle(b)
        lax.fori_loop(b * SPB, (b + 1) * SPB, w_step, 0)
        return carry

    lax.fori_loop(0, B, batch, 0)

    g8 = _rows8(g_v[...])
    dh = dh_s[...]
    outs = []

    def put(src, dst, i):
        cp = misc(src, dst, i)
        cp.start()
        outs.append(cp)

    put(out_v, out_hbm, 0)
    db1_v[...] = jnp.sum(du_s[...], axis=0).astype(BF)
    db2_v[...] = jnp.sum(g8, axis=0).astype(BF)
    put(db1_v, db1_hbm, 2)
    put(db2_v, db2_hbm, 3)

    wo_v[...] = _dot(o_s[...].astype(BF), dh.astype(BF), TN).astype(BF)
    put(wo_v, dwo_hbm, 5)
    w1_v[...] = _dot(y2_s[...].astype(BF), du_s[...].astype(BF), TN).astype(BF)
    put(w1_v, dw1_hbm, 6)
    w2_v[...] = _dot(hid_s[...].astype(BF), g8.astype(BF), TN).astype(BF)
    put(w2_v, dw2_hbm, 7)

    dq_all = dq_s[...].astype(BF)
    xn, r0 = _ln_fwd(_rows8(x_v[...]))
    dx8 = dh + _ln_bwd(_dot(dq_all, wq_v[...], NT), xn, r0)
    dx_v[...] = dx8[0:B].astype(BF)
    put(dx_v, dx_hbm, 1)
    wq_v[...] = _dot(xn.astype(BF), dq_all, TN).astype(BF)
    put(wq_v, dwq_hbm, 4)

    for slot in range(NS):
        wait_slot(slot)
    for cp in outs:
        cp.wait()


@jax.jit
def pallas_sequential_preLN__mha_block_cached__mixer_channel_mlp__decode_kernel(
    A_x: jax.Array,
    A_k_cache: jax.Array,
    A_v_cache: jax.Array,
    A_wq: jax.Array,
    A_wo: jax.Array,
    B_x: jax.Array,
    B_w1: jax.Array,
    B_b1: jax.Array,
    B_w2: jax.Array,
    B_b2: jax.Array,
    grad_out: jax.Array,
):
    del B_x
    any_spec = pl.BlockSpec(memory_space=pl.ANY)
    sds = jax.ShapeDtypeStruct
    out_shape = [
        sds((B, D), BF), sds((B, D), BF),
        sds((B, H, S, DH), BF), sds((B, H, S, DH), BF),
        sds((D, H * DH), BF), sds((H * DH, D), BF),
        sds((D, F), BF), sds((F,), BF), sds((F, D), BF), sds((D,), BF),
    ]
    vm = pltpu.VMEM
    scratch = [
        vm((NK, S, DH), BF), vm((NV, S, DH), BF), vm((NS, R // C, G, C, DH), BF),
        vm((D, H * DH), BF), vm((H * DH, D), BF), vm((D, F), BF), vm((F, D), BF),
        vm((B, D), BF), vm((B, D), BF), vm((F,), BF), vm((D,), BF),
        vm((2, B, NG, G, S), F32), vm((2, B, NG, G, DH), F32),
        vm((8, H * DH), F32), vm((2, NG, G, DH), F32), vm((8, H * DH), F32),
        vm((H, DH, DH), BF), vm((H, DH, DH), BF), vm((8, S), F32),
        vm((8, D), F32), vm((8, D), F32), vm((8, D), F32), vm((8, F), F32), vm((8, F), F32),
        vm((B, D), BF), vm((B, D), BF), vm((F,), BF), vm((D,), BF),
        pltpu.SemaphoreType.DMA((NK,)), pltpu.SemaphoreType.DMA((NK,)),
        pltpu.SemaphoreType.DMA((NS,)), pltpu.SemaphoreType.DMA((8,)),
    ]
    res = pl.pallas_call(
        _kernel,
        in_specs=[any_spec] * 10,
        out_specs=[any_spec] * 10,
        out_shape=out_shape,
        scratch_shapes=scratch,
        compiler_params=pltpu.CompilerParams(vmem_limit_bytes=120 * 1024 * 1024),
    )(A_x.reshape(B, D), A_k_cache, A_v_cache, A_wq, A_wo, B_w1, B_b1, B_w2, B_b2,
      grad_out.reshape(B, D))
    out, dx = res[0].reshape(B, 1, D), res[1].reshape(B, 1, D)
    return (out, dx) + tuple(res[2:])
```

```python
import jax
import jax.numpy as jnp
from jax import lax
import jax.experimental.pallas as pl
import jax.experimental.pallas.tpu as pltpu

BF = jnp.bfloat16
F32 = jnp.float32

B, H, S, DH, D, F = 2, 32, 8192, 128, 512, 1792
T = B * H
SCALE = DH ** -0.5
EPS = 1e-5
NOBC = True

NK = 3
NV = H + 1
NQ = 4
QR = S // NQ
FR = 16
VFR = 32
KBR = 128
VBR = 64
SSUB = 1024
MSUB = 512
NB = S // SSUB
NE = S // MSUB
NC = 1
NX = 16
NTICK = 23
NKF = NC + NTICK + NB
NKB = (QR - NKF * FR) // KBR
NVF = NE
NVB = (QR - NVF * VFR) // VBR
NEARLY = 2
assert NKF * FR + NKB * KBR == QR and NVF * VFR + NVB * VBR == QR
NVL = NVB - NE
assert NVL >= 0 and NVL + NKB <= NTICK <= NVB and NX <= NTICK

G = 8
SPH = 2
HG = G // SPH
SR = S // SPH
NG = H // HG
R = 512
C = 64
NN_ = SR // R
SPB = 2 * NG * NN_
NS = 12
NLEFT = 3
NDEF = 6
HP = NN_ // HG
DKV_SHAPE = (B, NG, G, SR, DH)
assert NDEF <= NN_

WQ_SHAPE = (8, D // 8, H * DH)
WO_SHAPE = (8, H * DH // 8, D)
W1_SHAPE = (4, D // 4, F)
W2_SHAPE = (4, F // 4, D)

NT = (((1,), (1,)), ((), ()))
NN = (((1,), (0,)), ((), ()))
TN = (((0,), (0,)), ((), ()))


def _dot(a, b, dims):
    return lax.dot_general(a, b, dims, preferred_element_type=F32)


def _ln_fwd(x):
    m = jnp.mean(x, axis=-1, keepdims=True)
    xc = x - m
    v = jnp.mean(xc * xc, axis=-1, keepdims=True)
    rstd = lax.rsqrt(v + EPS)
    return xc * rstd, rstd


def _ln_bwd(dy, y, rstd):
    m1 = jnp.mean(dy, axis=-1, keepdims=True)
    m2 = jnp.mean(dy * y, axis=-1, keepdims=True)
    return (dy - m1 - y * m2) * rstd


def _rows8(x2):
    return jnp.concatenate([x2.astype(F32), jnp.zeros((6, x2.shape[1]), F32)], axis=0)


def _flat(w3):
    return w3.reshape(w3.shape[0] * w3.shape[1], w3.shape[2])


def _kernel(x_hbm, k_hbm, v_hbm, wq_hbm, wo_hbm, w1_hbm, b1_hbm, w2_hbm, b2_hbm, g_hbm,
            out_hbm, dx_hbm, dk_hbm, dv_hbm, dwq_hbm, dwo_hbm, dw1_hbm, db1_hbm, dw2_hbm, db2_hbm,
            kbuf, vbuf, stage, wq_v, wo_v, w1_v, w2_v, x_v, g_v, b1_v, b2_v,
            coef, vec, o_s, hv, dq_s, mhi, mlo, s_s, p_s, mx_s,
            h1_s, dh_s, y2_s, du_s, hid_s, dhid_s,
            out_v, dx_v, db1_v, db2_v,
            ksem, vsem, wsem, msem):

    class Loader:
        def __init__(self, hbm, buf, nslot, sem, t, nfine, fine_rows, big_rows):
            self.src, self.dst, self.sem = hbm.at[t // H, t % H], buf.at[t % nslot], sem.at[t % NK]
            self.nfine, self.fine_rows, self.big_rows = nfine, fine_rows, big_rows

        def rows(self, row, n):
            if not isinstance(row, int):
                row = pl.multiple_of(row, 16)
            return pltpu.make_async_copy(
                self.src.at[:, pl.ds(row, n)], self.dst.at[:, pl.ds(row, n)], self.sem)

        def fine(self, f):
            return self.rows(f * self.fine_rows, self.fine_rows)

        def big(self, j):
            return self.rows(self.nfine * self.fine_rows + j * self.big_rows, self.big_rows)

    def k_load(t):
        return Loader(k_hbm, kbuf, NK, ksem, t, NKF, FR, KBR)

    def v_load(t):
        return Loader(v_hbm, vbuf, NV, vsem, t, NVF, VFR, VBR)

    def start_range(make, lo, hi, priority):
        def body(j, c):
            make(j).start(priority=priority)
            return c
        lax.fori_loop(lo, hi, body, 0)

    def start_if(cond, cp, priority):
        pl.when(cond)(lambda: cp.start(priority=priority))

    def wait_k(t):
        kl = k_load(t)
        for j in range(NKB):
            kl.big(j).wait()
        for f in range(NKF):
            kl.fine(f).wait()

    def misc(src, dst, i):
        return pltpu.make_async_copy(src, dst, msem.at[i])

    def issue_step(dst, b, g, n, slot):
        for c in range(R // C):
            row = pl.multiple_of(n * R + c * C, C)
            pltpu.make_async_copy(
                stage.at[slot, c],
                dst.at[b, g, :, pl.ds(row, C)],
                wsem.at[slot]).start()

    def wait_slot(slot):
        pltpu.make_async_copy(stage.at[slot], stage.at[slot], wsem.at[slot]).wait()

    def wait_piece(slot, c):
        pltpu.make_async_copy(stage.at[slot, c], stage.at[slot, c], wsem.at[slot]).wait()

    def scores(t, before_sub):
        h = t % H
        q8 = jnp.broadcast_to(vec[1, t // H, h // HG, pl.ds(h % HG, 1), :], (8, DH)).astype(BF)
        mx = None
        for u in range(NB):
            before_sub(u)
            r = u * SSUB
            sc = _dot(q8, kbuf[t % NK, r // QR, r % QR:r % QR + SSUB, :], NT)
            s_s[:, r:r + SSUB] = sc
            for tt in range(SSUB // DH):
                piece = sc[:, tt * DH:(tt + 1) * DH]
                mx = piece if mx is None else jnp.maximum(mx, piece)
        mx_s[...] = mx

    in_small = [misc(x_hbm, x_v, 0), misc(g_hbm, g_v, 1), misc(b1_hbm, b1_v, 2), misc(b2_hbm, b2_v, 3)]
    in_wq = misc(wq_hbm, wq_v, 4)
    in_wo = misc(wo_hbm, wo_v, 5)
    in_w = [misc(w1_hbm, w1_v, 6), misc(w2_hbm, w2_v, 7)]
    in_wq.start(priority=1)
    for cp in in_small:
        cp.start()
    start_range(k_load(0).big, 0, NKB, 1)
    start_range(k_load(0).fine, 0, NKF, 1)
    in_wo.start(priority=1)
    for cp in in_w:
        cp.start(priority=1)

    o_s[...] = jnp.zeros(o_s.shape, F32)
    dq_s[...] = jnp.zeros(dq_s.shape, F32)

    for cp in in_small:
        cp.wait()
    x8 = _rows8(x_v[...])
    h1_s[...] = x8
    xn, _ = _ln_fwd(x8)
    in_wq.wait()
    q_all = _dot(xn.astype(BF), _flat(wq_v[...]), NN).astype(BF).astype(F32)
    for bb in range(B):
        for h in range(H):
            vec[1, bb, h // HG, pl.ds(h % HG, 1), :] = q_all[bb:bb + 1, h * DH:(h + 1) * DH]
    wait_k(0)
    start_range(k_load(1).big, 0, NKB, 1)
    start_range(k_load(1).fine, 0, NKF, 1)
    start_range(v_load(0).fine, 0, NVF, 1)
    start_range(v_load(0).big, 0, NE, 1)
    scores(0, lambda u: None)
    in_wo.wait()

    row8 = lax.broadcasted_iota(jnp.int32, (8, DH), 0)

    def fwd_head(h, b):
        t = b * H + h
        g, i = h // HG, h % HG
        ks, vs = t % NK, t % NV
        col = pl.multiple_of(h * DH, DH)
        more1, more2 = t + 1 < T, t + 2 < T
        fresh = t != H
        go1, go2 = jnp.logical_and(more1, fresh), jnp.logical_and(more2, fresh)
        t1 = jnp.minimum(t + 1, T - 1)
        v_cur, v_nxt, k_nxt = v_load(t), v_load(t1), k_load(jnp.minimum(t + 2, T - 1))

        @pl.when(t == T - 1)
        def _():
            def issue_deferred(n, c):
                issue_step(dk_hbm, 0, NG - 1, n, (SPB - NN_ + n) % NS)
                return c
            lax.fori_loop(NN_ - NDEF, NN_, issue_deferred, 0)

        start_if(go2, k_nxt.fine(0), 0)
        m = jnp.broadcast_to(jnp.max(mx_s[...], axis=1, keepdims=True), (8, DH))

        last_slot = (SPB - NDEF - 1) % NS

        @pl.when(t == H)
        def _():
            for j in range(SPB - NS, SPB - NDEF - 1):
                wait_slot(j % NS)
            for c in range(R // C - NLEFT):
                wait_piece(last_slot, c)

        for f in range(NVF):
            v_cur.fine(f).wait()
        for j in range(NTICK, NVB):
            v_cur.big(j).wait()

        cc = S // NX

        def tick_starts(f):
            start_if(go2, k_nxt.fine(NC + f), 0)
            start_if(jnp.logical_and(go1, f < NVL), v_cur.big(jnp.minimum(NE + f, NVB - 1)), 1)
            j = f - jnp.where(fresh, NVL, -NEARLY)
            start_if(jnp.logical_and(more2, jnp.logical_and(j >= 0, j < NKB)),
                     k_nxt.big(jnp.clip(j, 0, NKB - 1)), 1)
            start_if(jnp.logical_and(t == T - 2, f >= NTICK - NVL),
                     v_nxt.big(jnp.clip(NVB - NTICK + f, 0, NVB - 1)), 1)

        def tick_exp(f, tot):
            tick_starts(f)
            for tt in range(cc // DH):
                r = pl.multiple_of(f * cc + tt * DH, DH)
                e = jnp.exp((s_s[:, pl.ds(r, DH)] - m) * SCALE)
                p_s[:, pl.ds(r, DH)] = e
                tot = tot + e
            v_cur.big(f).wait()
            return tot

        def tick(f, c):
            tick_starts(f)
            v_cur.big(f).wait()
            return c

        tot = lax.fori_loop(0, NX, tick_exp, jnp.zeros((8, DH), F32))
        lax.fori_loop(NX, NTICK, tick, 0)
        pl.when(more1)(lambda: wait_k(t1))

        inv = 1.0 / jnp.sum(tot, axis=1, keepdims=True)
        for z in range(SPH):
            coef[0, b, g, pl.ds(i * SPH + z, 1), :] = p_s[0:1, z * SR:(z + 1) * SR] * inv[0:1]
        acc = jnp.zeros((DH + 16, DH), F32)
        kb = jnp.zeros((16, DH), F32)
        for u in range(NE):
            start_if(more1, v_nxt.fine(u), 0)
            start_if(more1, v_nxt.big(u), 1)
            r = u * MSUB
            q, r0 = r // QR, r % QR
            kc = kbuf[ks, q, r0:r0 + MSUB, :]
            p8 = p_s[:, r:r + MSUB]
            p_hi = p8.astype(BF)
            p_lo = (p8 - p_hi.astype(F32)).astype(BF)
            p16 = jnp.concatenate([p_hi, p_lo], axis=0)
            a = (kc.astype(F32).T * p_s[0:1, r:r + MSUB]).astype(BF)
            acc = acc + _dot(jnp.concatenate([a, p16], axis=0), vbuf[vs, q, r0:r0 + MSUB, :], NN)
            kb = kb + _dot(p16, kc, NN)

        scores(t1, lambda u: start_if(more2, k_nxt.fine(NC + NTICK + u), 0))

        mt = acc[0:DH] * inv[0:1]
        mt_hi = mt.astype(BF)
        mhi[h] = mt_hi
        mlo[h] = (mt - mt_hi.astype(F32)).astype(BF)
        o8 = (acc[DH:DH + 8] + acc[DH + 8:DH + 16]) * inv
        ob = jnp.where(row8 == b, o8, 0.0)
        o_s[:, pl.ds(col, DH)] += ob
        hps = WO_SHAPE[1] // DH
        wo_h = wo_v[h // hps, pl.ds(pl.multiple_of((h % hps) * DH, DH), DH), :]
        h1_s[...] += _dot(ob.astype(BF), wo_h, NN)
        hv[0, g, pl.ds(i, 1), :] = o8[0:1]
        hv[1, g, pl.ds(i, 1), :] = (kb[0:1] + kb[8:9]) * inv[0:1]

        @pl.when(t == H)
        def _():
            for c in range(R // C - NLEFT, R // C):
                wait_piece(last_slot, c)

        @pl.when(t == H // 2)
        def _():
            for cp in in_w:
                cp.wait()
            dhid_s[...] = _dot(_rows8(g_v[...]).astype(BF), _flat(w2_v[...]), NT)

        return b

    def middle():
        y1, r1 = _ln_fwd(h1_s[...])
        y2, r2 = _ln_fwd(y1)
        u = _dot(y2.astype(BF), _flat(w1_v[...]), NN) + b1_v[...].astype(F32).reshape(1, F)
        c0 = (2.0 / jnp.pi) ** 0.5
        th = jnp.tanh(c0 * (u + 0.044715 * (u * u * u)))
        dgelu = 0.5 * (1.0 + th) + 0.5 * u * (1.0 - th * th) * (c0 * (1.0 + 3 * 0.044715 * (u * u)))
        du = dhid_s[...] * dgelu
        dy2 = _dot(du.astype(BF), _flat(w1_v[...]), NT)
        dh_s[...] = _rows8(g_v[...]) + _ln_bwd(_ln_bwd(dy2, y2, r2), y1, r1)
        y2_s[...] = y2
        du_s[...] = du
        hid_s[...] = 0.5 * u * (1.0 + th)

    eye = (lax.broadcasted_iota(jnp.int32, (DH, DH), 0) == lax.broadcasted_iota(jnp.int32, (DH, DH), 1))

    def fill_slot(kind, b, g, n):
        j = b * SPB + (2 * g + kind) * NN_ + n
        slot = j % NS
        drained = jnp.logical_and(j >= SPB, j < SPB + NS - NDEF)

        @pl.when(jnp.logical_and(j >= NS, jnp.logical_not(drained)))
        def _():
            wait_slot(slot)

        for i in range(HG):
            w = jnp.broadcast_to(vec[kind, b, g, pl.ds(i, 1), :], (DH, DH)).astype(BF)
            tiles = []
            for z in range(SPH):
                for tt in range(R // DH):
                    r = pl.multiple_of(n * R + tt * DH, DH)
                    cf = coef[kind, b, g, pl.ds(i * SPH + z, 1), pl.ds(r, DH)]
                    tiles.append(jnp.where(eye, cf, 0.0).astype(BF))
            res = _dot(jnp.concatenate(tiles, axis=0), w, NN).astype(BF)
            for z in range(SPH):
                stage[slot, :, i * SPH + z] = res[z * R:(z + 1) * R].reshape(R // C, C, DH)
        return j, slot

    def bwd_head(b, g, i):
        h = g * HG + i
        col = pl.multiple_of(h * DH, DH)
        vs = (b * H + h) % NV
        do_row = vec[0, b, g, pl.ds(i, 1), :]
        dsum = jnp.sum(do_row * hv[0, g, pl.ds(i, 1), :], axis=1, keepdims=True)
        do8 = jnp.broadcast_to(do_row, (8, DH)).astype(BF)
        dq = _dot(do8, mhi[h], NT) + _dot(do8, mlo[h], NT)
        dq = (dq - dsum * hv[1, g, pl.ds(i, 1), :]) * SCALE
        dq_s[:, pl.ds(col, DH)] += jnp.where(row8 == b, dq, 0.0)
        dp = _dot(do8, _flat(vbuf[vs]), NT)
        for z in range(SPH):
            row = pl.ds(i * SPH + z, 1)
            coef[1, b, g, row, :] = coef[0, b, g, row, :] * ((dp[0:1, z * SR:(z + 1) * SR] - dsum) * SCALE)

    def group(g, b):
        spg = HG * DH // WO_SHAPE[1]
        do_g = _dot(dh_s[...].astype(BF), _flat(wo_v[pl.ds(g * spg, spg)]), NT).astype(BF).astype(F32)
        row = lax.broadcasted_iota(jnp.int32, do_g.shape, 0)
        do_b = jnp.sum(jnp.where(row == b, do_g, 0.0), axis=0, keepdims=True)
        for i in range(HG):
            vec[0, b, g, pl.ds(i, 1), :] = do_b[:, i * DH:(i + 1) * DH]

        def dv_step(n, c):
            _, slot = fill_slot(0, b, g, n)
            issue_step(dv_hbm, b, g, n, slot)

            @pl.when(n % HP == HP - 1)
            def _():
                bwd_head(b, g, n // HP)
            return c

        def dk_step(n, c):
            j, slot = fill_slot(1, b, g, n)

            @pl.when(jnp.logical_or(j < SPB - NDEF, j >= SPB))
            def _():
                issue_step(dk_hbm, b, g, n, slot)
            return c

        lax.fori_loop(0, NN_, dv_step, 0)
        lax.fori_loop(0, NN_, dk_step, 0)
        return b

    def batch(b, carry):
        lax.fori_loop(0, H, fwd_head, b)

        @pl.when(b == 0)
        def _():
            start_range(v_load(H).big, NE, NVB, 1)
            start_range(k_load(H + 2).fine, 0, NC + NTICK, 1)
            start_range(k_load(H + 2).big, 0, NEARLY, 1)

        middle()
        lax.fori_loop(0, NG, group, b)
        return carry

    lax.fori_loop(0, B, batch, 0)

    g8 = _rows8(g_v[...])
    dh = dh_s[...]
    outs = []

    def put(src, dst, i):
        cp = misc(src, dst, i)
        cp.start()
        outs.append(cp)

    def piece(src, dst, i, j, cols):
        per_row = src.shape[2] // cols
        row = pl.multiple_of((j // per_row) * 16, 16)
        cs = pl.ds(pl.multiple_of((j % per_row) * cols, DH), cols) if per_row > 1 else slice(None)
        return misc(src.at[:, pl.ds(row, 16), cs], dst.at[:, pl.ds(row, 16), cs], i)

    out8 = h1_s[...] + _dot(hid_s[...].astype(BF), _flat(w2_v[...]), NN) + b2_v[...].astype(F32).reshape(1, D)
    out_v[...] = out8[0:B].astype(BF)
    put(out_v, out_hbm, 0)
    db1_v[...] = jnp.sum(du_s[...], axis=0).astype(BF)
    db2_v[...] = jnp.sum(g8, axis=0).astype(BF)
    put(db1_v, db1_hbm, 2)
    put(db2_v, db2_hbm, 3)

    wo_v[...] = _dot(o_s[...].astype(BF), dh.astype(BF), TN).astype(BF).reshape(WO_SHAPE)
    start_range(lambda j: piece(wo_v, dwo_hbm, 5, j, D), 0, WO_SHAPE[1] // 16, 0)

    w1_v[...] = _dot(y2_s[...].astype(BF), du_s[...].astype(BF), TN).astype(BF).reshape(W1_SHAPE)
    w2_v[...] = _dot(hid_s[...].astype(BF), g8.astype(BF), TN).astype(BF).reshape(W2_SHAPE)

    def mlp_pieces(j, c):
        for jj in range(4):
            piece(w1_v, dw1_hbm, 6, 4 * j + jj, F // 2).start()
            piece(w2_v, dw2_hbm, 7, 7 * j + 2 * jj, D).start()
            if jj < 3:
                piece(w2_v, dw2_hbm, 7, 7 * j + 2 * jj + 1, D).start()
        return c

    lax.fori_loop(0, 4, mlp_pieces, 0)

    dq_all = dq_s[...].astype(BF)
    xn, r0 = _ln_fwd(_rows8(x_v[...]))
    dx8 = dh + _ln_bwd(_dot(dq_all, _flat(wq_v[...]), NT), xn, r0)
    dx_v[...] = dx8[0:B].astype(BF)
    put(dx_v, dx_hbm, 1)
    wq_v[...] = _dot(xn.astype(BF), dq_all, TN).astype(BF).reshape(WQ_SHAPE)
    start_range(lambda j: piece(wq_v, dwq_hbm, 4, j, 512), 0, (WQ_SHAPE[1] // 16) * (H * DH // 512), 0)

    for slot in range(NS):
        wait_slot(slot)
    for cp in outs:
        cp.wait()
    for i, buf in ((5, wo_v), (6, w1_v), (7, w2_v), (4, wq_v)):
        misc(buf, buf, i).wait()


@jax.jit
def pallas_sequential_preLN__mha_block_cached__mixer_channel_mlp__decode_kernel(
    A_x: jax.Array,
    A_k_cache: jax.Array,
    A_v_cache: jax.Array,
    A_wq: jax.Array,
    A_wo: jax.Array,
    B_x: jax.Array,
    B_w1: jax.Array,
    B_b1: jax.Array,
    B_w2: jax.Array,
    B_b2: jax.Array,
    grad_out: jax.Array,
):
    del B_x
    any_spec = pl.BlockSpec(memory_space=pl.ANY)
    sds = jax.ShapeDtypeStruct
    out_shape = [
        sds((B, D), BF), sds((B, D), BF),
        sds(DKV_SHAPE, BF), sds(DKV_SHAPE, BF),
        sds(WQ_SHAPE, BF), sds(WO_SHAPE, BF),
        sds(W1_SHAPE, BF), sds((F,), BF), sds(W2_SHAPE, BF), sds((D,), BF),
    ]
    vm = pltpu.VMEM
    scratch = [
        vm((NK, NQ, QR, DH), BF), vm((NV, NQ, QR, DH), BF), vm((NS, R // C, G, C, DH), BF),
        vm(WQ_SHAPE, BF), vm(WO_SHAPE, BF), vm(W1_SHAPE, BF), vm(W2_SHAPE, BF),
        vm((B, D), BF), vm((B, D), BF), vm((F,), BF), vm((D,), BF),
        vm((2, B, NG, G, SR), F32), vm((2, B, NG, 8, DH), F32),
        vm((8, H * DH), F32), vm((2, NG, 8, DH), F32), vm((8, H * DH), F32),
        vm((H, DH, DH), BF), vm((H, DH, DH), BF), vm((8, S), F32), vm((8, S), F32), vm((8, DH), F32),
        vm((8, D), F32), vm((8, D), F32), vm((8, D), F32), vm((8, F), F32), vm((8, F), F32), vm((8, F), F32),
        vm((B, D), BF), vm((B, D), BF), vm((F,), BF), vm((D,), BF),
        pltpu.SemaphoreType.DMA((NK,)), pltpu.SemaphoreType.DMA((NK,)),
        pltpu.SemaphoreType.DMA((NS,)), pltpu.SemaphoreType.DMA((8,)),
    ]
    res = pl.pallas_call(
        _kernel,
        in_specs=[any_spec] * 10,
        out_specs=[any_spec] * 10,
        out_shape=out_shape,
        scratch_shapes=scratch,
        compiler_params=pltpu.CompilerParams(vmem_limit_bytes=120 * 1024 * 1024, disable_bounds_checks=NOBC),
    )(A_x.reshape(B, D), A_k_cache.reshape(B, H, NQ, QR, DH), A_v_cache.reshape(B, H, NQ, QR, DH),
      A_wq.reshape(WQ_SHAPE), A_wo.reshape(WO_SHAPE), B_w1.reshape(W1_SHAPE), B_b1,
      B_w2.reshape(W2_SHAPE), B_b2, grad_out.reshape(B, D))
    out, dx, dk, dv, dwq, dwo, dw1, db1, dw2, db2 = res
    return (out.reshape(B, 1, D), dx.reshape(B, 1, D), dk.reshape(B, H, S, DH), dv.reshape(B, H, S, DH),
            dwq.reshape(D, H * DH), dwo.reshape(H * DH, D), dw1.reshape(D, F), db1, dw2.reshape(F, D), db2)
```

```python
import jax
import jax.numpy as jnp
from jax import lax
import jax.experimental.pallas as pl
import jax.experimental.pallas.tpu as pltpu

BF = jnp.bfloat16
F32 = jnp.float32

B, H, S, DH, D, F = 2, 32, 8192, 128, 512, 1792
SCALE = DH ** -0.5
EPS = 1e-5
NOBC = True

G = 8
SPH = 2
HG = G // SPH
SR = S // SPH
NG = H // HG
SHIFT = 1
GA = SPH
GB = G - GA
KV_SHAPE = (B, H * SPH, SR, DH)
assert SHIFT * SPH <= GA

QR = S // G
TPG = SR // QR
TPB = NG * TPG
T = B * TPB
NK = 3
NV = TPB + 1
BL = 64
FR = 8
NBL = QR // BL
LAG = 3
AHEAD = 4
MSUB = 512
NE = S // MSUB
FSKIP = (3, 10)
WOTICK = 6
assert NE == NBL and len(FSKIP) >= 1

R = 512
C = 64
NN_ = SR // R
SPB = 2 * NG * NN_
NS = 12
NLEFT = 1
NDEF = 8
assert NDEF <= NN_ and NN_ == G

WQ_SHAPE = (8, D // 8, H * DH)
WO_SHAPE = (NG, HG * DH, D)
W1_SHAPE = (4, D // 4, F)
W2_SHAPE = (4, F // 4, D)

NT = (((1,), (1,)), ((), ()))
NN = (((1,), (0,)), ((), ()))
TN = (((0,), (0,)), ((), ()))


def _dot(a, b, dims):
    return lax.dot_general(a, b, dims, preferred_element_type=F32)


def _ln_fwd(x):
    m = jnp.mean(x, axis=-1, keepdims=True)
    xc = x - m
    v = jnp.mean(xc * xc, axis=-1, keepdims=True)
    rstd = lax.rsqrt(v + EPS)
    return xc * rstd, rstd


def _ln_bwd(dy, y, rstd):
    m1 = jnp.mean(dy, axis=-1, keepdims=True)
    m2 = jnp.mean(dy * y, axis=-1, keepdims=True)
    return (dy - m1 - y * m2) * rstd


def _rows8(x2):
    return jnp.concatenate([x2.astype(F32), jnp.zeros((6, x2.shape[1]), F32)], axis=0)


def _flat(w3):
    return w3.reshape(w3.shape[0] * w3.shape[1], w3.shape[2])


def _aligned(x, n):
    return x if isinstance(x, int) else pl.multiple_of(x, n)


class _Blocks:
    def __init__(self, src, dst, sem, fsem, block, axis, fine_size):
        self.src, self.dst, self.sem, self.fsem = src, dst, sem, fsem
        self.block, self.axis, self.fine_size = block, axis, fine_size
        self.grid = [n // m for n, m in zip(dst.shape, block)]
        self.n = self.grid[0] * self.grid[1] * self.grid[2]

    def _part(self, j, offset, size, sem):
        at, inner = [], self.n
        for ax, align in enumerate((1, 8, DH)):
            outer, inner = inner, inner // self.grid[ax]
            pos = 0
            if self.grid[ax] > 1:
                pos = j if outer == self.n else j % outer
                pos = pos if inner == 1 else pos // inner
            lo = pos * self.block[ax] + (offset if ax == self.axis else 0)
            at.append(pl.ds(_aligned(lo, align), size if ax == self.axis else self.block[ax]))
        return pltpu.make_async_copy(self.src.at[tuple(at)], self.dst.at[tuple(at)], sem)

    def big(self, j):
        return self._part(j, 0, self.block[self.axis] - self.fine_size, self.sem)

    def fine(self, j):
        return self._part(j, self.block[self.axis] - self.fine_size, self.fine_size, self.fsem)

    def wait_big(self, lo, hi):
        for j in range(lo, hi):
            self.big(j).wait()

    def wait_fine(self):
        for j in range(self.n):
            self.fine(j).wait()


class _Pair:
    def __init__(self, first, second):
        self.copies = (first, second)

    def start(self, priority=0):
        for cp in self.copies:
            cp.start(priority=priority)

    def wait(self):
        for cp in self.copies:
            cp.wait()


class _BlockPairs(_Blocks):
    def __init__(self, first, second):
        self.parts, self.n = (first, second), first.n

    def big(self, j):
        return _Pair(*[p.big(j) for p in self.parts])

    def fine(self, j):
        return _Pair(*[p.fine(j) for p in self.parts])


def _head(g, i):
    return (g * HG + i + H - SHIFT) % H


def _segments(g):
    s0 = g * G - SHIFT * SPH
    return ((pl.ds((s0 + H * SPH) % (H * SPH), GA), pl.ds(0, GA)), (pl.ds(s0 + GA, GB), pl.ds(GA, GB)))


def _start_if(cond, copy, priority):
    pl.when(cond)(lambda: copy.start(priority=priority))


def _kernel(x_hbm, k_hbm, v_hbm, wq_hbm, wo_hbm, w1_hbm, b1_hbm, w2_hbm, b2_hbm, g_hbm,
            out_hbm, dx_hbm, dk_hbm, dv_hbm, dwq_hbm, dwo_hbm, dw1_hbm, db1_hbm, dw2_hbm, db2_hbm,
            kbuf, vbuf, stage, wq_v, wo_v, w1_v, w2_v, x_v, g_v, b1_v, b2_v,
            coef, vec, o_s, hv, dq_s, mhi, mlo, s_s, p_s, mx_s, m_s, l_s, macc, kacc,
            h1_s, dh_s, y2_s, du_s, hid_s, dhid_s,
            out_v, dx_v, db1_v, db2_v,
            ksem, vsem, wsem, msem):
    both = jnp.logical_and
    row8 = lax.broadcasted_iota(jnp.int32, (8, DH), 0)

    def tile_load(hbm, buf, nslot, sem, t):
        rows = pl.ds(_aligned((t % TPG) * QR, QR), QR)
        return _BlockPairs(*[
            _Blocks(hbm.at[t // TPB, far, rows], buf.at[t % nslot, near],
                    sem.at[t % NK], sem.at[NK + t % NK], (near.size, BL, DH), 1, FR)
            for far, near in _segments((t % TPB) // TPG)])

    def k_load(t):
        return tile_load(k_hbm, kbuf, NK, ksem, t)

    def v_load(t):
        return tile_load(v_hbm, vbuf, NV, vsem, t)

    def misc(src, dst, i):
        return pltpu.make_async_copy(src, dst, msem.at[i])

    def issue_step(dst, b, g, n, slot):
        def issue(segments):
            for c in range(R // C):
                row = pl.multiple_of(n * R + c * C, C)
                for far, near in segments:
                    pltpu.make_async_copy(
                        stage.at[slot, c, near], dst.at[b, far, pl.ds(row, C)], wsem.at[slot]).start()

        if isinstance(g, int) and g > 0:
            issue([(pl.ds(g * G - SHIFT * SPH, G), pl.ds(0, G))])
        else:
            pl.when(g == 0)(lambda: issue(_segments(0)))
            pl.when(g > 0)(lambda: issue([(pl.ds(jnp.maximum(g * G - SHIFT * SPH, 0), G), pl.ds(0, G))]))

    def wait_slot(slot):
        pltpu.make_async_copy(stage.at[slot], stage.at[slot], wsem.at[slot]).wait()

    def wait_pieces(slot, lo, hi):
        for c in range(lo, hi):
            pltpu.make_async_copy(stage.at[slot, c], stage.at[slot, c], wsem.at[slot]).wait()

    def wo_group(g):
        cut = (HG - SHIFT) * DH
        if SHIFT == 0:
            return wo_v[g]
        return jnp.concatenate([wo_v[(g + NG - 1) % NG, cut:, :], wo_v[g, :cut, :]], axis=0)

    def group_cols(g):
        return pl.ds(_aligned(g * (HG * DH), HG * DH), HG * DH)

    def stream_scores(t, st):
        q_row = vec[1, t // TPB, (t % TPB) // TPG, pl.ds(st // SPH, 1), :]
        sc = _dot(jnp.broadcast_to(q_row, (8, DH)).astype(BF), kbuf[t % NK, st], NT)
        s_s[:, pl.ds(_aligned(st * QR, QR), QR)] = sc
        mx = sc[:, 0:DH]
        for tt in range(1, QR // DH):
            mx = jnp.maximum(mx, sc[:, tt * DH:(tt + 1) * DH])
        mx_s[st] = mx

    def add_attention(b, g):
        o_g = jnp.concatenate([jnp.where(row8 == b, hv[0, g, i:i + 1, :], 0.0) for i in range(HG)], axis=1)
        h1_s[...] += _dot(o_g.astype(BF), wo_group(g), NN)

    in_small = [misc(x_hbm, x_v, 0), misc(g_hbm, g_v, 1), misc(b1_hbm, b1_v, 2), misc(b2_hbm, b2_v, 3)]
    wq_l = _Blocks(wq_hbm, wq_v, msem.at[4], msem.at[8], (8, 8, 1024), 2, DH)
    wo_l = _Blocks(wo_hbm, wo_v, msem.at[5], msem.at[9], (4, 32, D), 1, 8)
    w1_l = _Blocks(w1_hbm, w1_v, msem.at[6], msem.at[10], (4, 8, F), 2, 2 * DH)
    w2_l = _Blocks(w2_hbm, w2_v, msem.at[7], msem.at[11], (4, 32, D), 1, 8)
    lag, depth = LAG + 1, LAG + 1 + AHEAD

    def paced(cur, nxt, count, work=None):
        def body(f, c):
            cur.big(f).wait()
            jf, jb = f + lag, f + depth
            _start_if(jf < cur.n, cur.fine(jnp.minimum(jf, cur.n - 1)), 0)
            _start_if(jf >= cur.n, nxt.fine(jnp.maximum(jf - cur.n, 0)), 0)
            _start_if(jb < cur.n, cur.big(jnp.minimum(jb, cur.n - 1)), 1)
            _start_if(jb >= cur.n, nxt.big(jnp.maximum(jb - cur.n, 0)), 1)
            if work is not None:
                pl.when(f % 2 == 0)(lambda: work(f // 2))
            return c
        lax.fori_loop(0, count, body, 0)

    for j in range(depth):
        wq_l.big(j).start(priority=1)
        if j == 0:
            for cp in in_small:
                cp.start()
        if j < lag:
            wq_l.fine(j).start()

    o_s[...] = jnp.zeros(o_s.shape, F32)
    dq_s[...] = jnp.zeros(dq_s.shape, F32)

    for cp in in_small:
        cp.wait()
    x8 = _rows8(x_v[...])
    h1_s[...] = x8
    y2_s[...] = _ln_fwd(x8)[0]

    def q_group(g):
        q_g = _dot(y2_s[...].astype(BF), _flat(wq_v[:, :, group_cols(g)]), NN).astype(BF).astype(F32)
        for bb in range(B):
            for i in range(HG):
                gg, ii = (g, i + SHIFT) if i + SHIFT < HG else ((g + 1) % NG, i + SHIFT - HG)
                vec[1, bb, gg, ii:ii + 1, :] = q_g[bb:bb + 1, i * DH:(i + 1) * DH]

    def dhid_part(j):
        @pl.when(j < W2_SHAPE[0])
        def _():
            jj = jnp.minimum(j, W2_SHAPE[0] - 1)
            dhid_s[jj] = _dot(_rows8(g_v[...]).astype(BF), w2_v[jj], NT)

    paced(wq_l, k_load(0), wq_l.n)
    wq_l.wait_fine()
    paced(k_load(0), w2_l, NBL, q_group)
    k_load(0).wait_fine()
    paced(w2_l, w1_l, w2_l.n)
    w2_l.wait_fine()
    paced(w1_l, wo_l, w1_l.n, lambda st: stream_scores(0, st))
    paced(wo_l, k_load(1), wo_l.n, dhid_part)
    w1_l.wait_fine()
    paced(k_load(1), v_load(0), NBL)
    wo_l.wait_fine()
    paced(v_load(0), k_load(2), NBL - lag)

    def by_head(vals):
        res = vals[HG - 1]
        for i in range(HG - 2, -1, -1):
            res = jnp.where(row8 < (i + 1) * SPH, vals[i], res)
        return res

    def fwd_tile(tb, b):
        t = b * TPB + tb
        g, rho = tb // TPG, tb % TPG
        first, last = rho == 0, rho == TPG - 1
        ks, vs = t % NK, t % NV
        more1, more2, more3 = t + 1 < T, t + 2 < T, t + 3 < T
        tail = t == T - 2
        go2 = both(more2, t != TPB)
        t1 = jnp.minimum(t + 1, T - 1)
        v0, v1, v_end = v_load(t), v_load(t1), v_load(T - 1)
        k1, k2, k3 = k_load(t1), k_load(jnp.minimum(t + 2, T - 1)), k_load(jnp.minimum(t + 3, T - 1))
        last_slot = (SPB - NDEF - 1) % NS
        cc = S // NBL

        def starts(f):
            jb = f + AHEAD
            jb_cur = jnp.minimum(jb, NBL - 1)
            _start_if(go2, k2.fine(f), 0)
            _start_if(tail, v_end.fine(f), 0)
            _start_if(both(go2, jb < NBL), k2.big(jb_cur), 1)
            _start_if(both(go2, jb >= NBL), v1.big(jnp.maximum(jb - NBL, 0)), 1)
            _start_if(both(tail, jb < NBL), v_end.big(jb_cur), 1)

        _start_if(both(more1, tb > 0), v0.fine(NBL - 1), 0)
        pl.when(both(more1, t > 0))(lambda: v0.wait_big(0, NBL - lag))
        pl.when(more1)(v0.big(NBL - lag).wait)
        starts(0)

        alpha = []
        for i in range(HG):
            mx = mx_s[i * SPH]
            for z in range(1, SPH):
                mx = jnp.maximum(mx, mx_s[i * SPH + z])
            m_blk = jnp.broadcast_to(jnp.max(mx, axis=1, keepdims=True), (8, DH))
            m_old = jnp.where(first, m_blk, m_s[i])
            m_new = jnp.maximum(m_old, m_blk)
            m_s[i] = m_new
            alpha.append(jnp.exp((m_old - m_new) * SCALE))

        def tick_exp(f, c):
            m = m_s[f // (NBL // HG)]
            for tt in range(cc // DH):
                r = pl.multiple_of(f * cc + tt * DH, DH)
                p_s[:, pl.ds(r, DH)] = jnp.exp((s_s[:, pl.ds(r, DH)] - m) * SCALE)

            @pl.when(both(f == WOTICK, both(first, g > 0)))
            def _():
                add_attention(b, jnp.maximum(g - 1, 0))

            j = jnp.maximum(f - LAG, 0)
            pl.when(f < LAG)(v0.big(jnp.minimum(NBL - LAG + f, NBL - 1)).wait)
            pl.when(both(f >= LAG, more2))(k2.big(j).wait)
            pl.when(both(f >= LAG, tail))(v_end.big(j).wait)
            pl.when(f + 1 < NBL)(lambda: starts(jnp.minimum(f + 1, NBL - 1)))
            return c

        lax.fori_loop(0, NBL, tick_exp, 0)
        v0.wait_fine()
        pl.when(both(more1, t > 0))(lambda: k1.wait_big(NBL - LAG, NBL))
        pl.when(more1)(k1.wait_fine)

        @pl.when(tail)
        def _():
            def issue_deferred(n, c):
                issue_step(dk_hbm, 0, NG - 1, n, (SPB - NN_ + n) % NS)
                return c
            lax.fori_loop(NN_ - NDEF, NN_, issue_deferred, 0)

        @pl.when(t == TPB)
        def _():
            for j in range(SPB - NS, SPB - NDEF - 1):
                wait_slot(j % NS)
            wait_pieces(last_slot, 0, R // C - NLEFT)
            for j in range(AHEAD):
                v_load(TPB + 1).big(j).start(priority=1)

        fin = []
        for i in range(HG):
            acc = jnp.where(first, 0.0, macc[i] * alpha[i][0:1])
            kb = jnp.where(first, 0.0, kacc[i] * alpha[i][0:1])
            tot = jnp.where(first, 0.0, l_s[i] * alpha[i])
            for u in range(i * NE // HG, (i + 1) * NE // HG):
                if u not in FSKIP:
                    _start_if(more2, v1.fine(u - sum(x < u for x in FSKIP)), 0)
                if u + AHEAD < NBL:
                    _start_if(more2, v1.big(u + AHEAD), 1)
                else:
                    _start_if(t == T - 3, v_end.big(u + AHEAD - NBL), 1)
                r = u * MSUB
                st, r0 = r // QR, r % QR
                kc = kbuf[ks, st, r0:r0 + MSUB, :]
                p8 = p_s[:, r:r + MSUB]
                for tt in range(MSUB // DH):
                    tot = tot + p8[:, tt * DH:(tt + 1) * DH]
                p_hi = p8.astype(BF).astype(F32)
                p16 = jnp.concatenate([p_hi, p8 - p_hi], axis=0)
                a = kc.astype(F32).T * p_s[0:1, r:r + MSUB]
                lhs = jnp.concatenate([a, p16], axis=0).astype(BF)
                acc = acc + _dot(lhs, vbuf[vs, st, r0:r0 + MSUB, :], NN)
                kb = kb + _dot(p16.astype(BF), kc, NN)
                if u == NE - 1:
                    for j in range(NE - len(FSKIP), NBL - 1):
                        _start_if(more2, v1.fine(j), 0)
                    for j in range(AHEAD):
                        _start_if(more3, k3.big(j), 1)
                if u % (NE // G) == NE // G - 1:
                    stream_scores(t1, u // (NE // G))
            macc[i] = acc
            kacc[i] = kb
            l_s[i] = tot
            inv = jnp.broadcast_to(1.0 / jnp.sum(tot, axis=1, keepdims=True), (8, DH))
            mt = acc[0:DH] * inv[0:1]
            mt_hi = mt.astype(BF)
            mhi[g * HG + i] = mt_hi
            mlo[g * HG + i] = (mt - mt_hi.astype(F32)).astype(BF)
            o8 = (acc[DH:DH + 8] + acc[DH + 8:DH + 16]) * inv
            hv[0, g, i:i + 1, :] = o8[0:1]
            hv[1, g, i:i + 1, :] = (kb[0:1] + kb[8:9]) * inv[0:1]
            col = pl.ds(pl.multiple_of(_head(g, i) * DH, DH), DH)
            o_s[:, col] = jnp.where(row8 == b, o8, o_s[:, col])
            fin.append(jnp.where(last, inv, 1.0))

        f_new = by_head(fin)
        f_old = by_head(alpha) * f_new
        for tt in range((SR - QR) // DH):
            coef[0, b, g, :, tt * DH:(tt + 1) * DH] *= f_old
        for tt in range(QR // DH):
            blk = p_s[:, (G - 1) * QR + tt * DH:(G - 1) * QR + (tt + 1) * DH]
            for st in range(G - 2, -1, -1):
                blk = jnp.where(row8 == st, p_s[:, st * QR + tt * DH:st * QR + (tt + 1) * DH], blk)
            coef[0, b, g, :, pl.ds(pl.multiple_of(rho * QR + tt * DH, DH), DH)] = blk * f_new

        pl.when(t == TPB)(lambda: wait_pieces(last_slot, R // C - NLEFT, R // C))
        return b

    def middle(b):
        add_attention(b, NG - 1)
        y1, r1 = _ln_fwd(h1_s[...])
        y2, r2 = _ln_fwd(y1)
        u = _dot(y2.astype(BF), _flat(w1_v[...]), NN) + b1_v[...].astype(F32).reshape(1, F)
        c0 = (2.0 / jnp.pi) ** 0.5
        th = jnp.tanh(c0 * (u + 0.044715 * (u * u * u)))
        dgelu = 0.5 * (1.0 + th) + 0.5 * u * (1.0 - th * th) * (c0 * (1.0 + 3 * 0.044715 * (u * u)))
        du = jnp.concatenate([dhid_s[j] for j in range(W2_SHAPE[0])], axis=1) * dgelu
        dy2 = _dot(du.astype(BF), _flat(w1_v[...]), NT)
        dh_s[...] = _rows8(g_v[...]) + _ln_bwd(_ln_bwd(dy2, y2, r2), y1, r1)
        y2_s[...] = y2
        du_s[...] = du
        hid_s[...] = 0.5 * u * (1.0 + th)

    eye = (lax.broadcasted_iota(jnp.int32, (DH, DH), 0) == lax.broadcasted_iota(jnp.int32, (DH, DH), 1))

    def fill_slot(kind, b, g, n):
        j = b * SPB + (2 * g + kind) * NN_ + n
        slot = j % NS
        drained = both(j >= SPB, j < SPB + NS - NDEF)
        pl.when(both(j >= NS, jnp.logical_not(drained)))(lambda: wait_slot(slot))

        for i in range(HG):
            w = jnp.broadcast_to(vec[kind, b, g, i:i + 1, :], (DH, DH)).astype(BF)
            tiles = []
            for z in range(SPH):
                for tt in range(R // DH):
                    r = pl.multiple_of(n * R + tt * DH, DH)
                    cf = coef[kind, b, g, pl.ds(i * SPH + z, 1), pl.ds(r, DH)]
                    tiles.append(jnp.where(eye, cf, 0.0).astype(BF))
            res = _dot(jnp.concatenate(tiles, axis=0), w, NN).astype(BF)
            for z in range(SPH):
                stage[slot, :, i * SPH + z] = res[z * R:(z + 1) * R].reshape(R // C, C, DH)
        return j, slot

    def bwd_stream(b, g, st):
        i = st // SPH
        h = g * HG + i
        col = pl.ds(pl.multiple_of(_head(g, i) * DH, DH), DH)
        do_row = vec[0, b, g, pl.ds(i, 1), :]
        dsum = jnp.sum(do_row * hv[0, g, pl.ds(i, 1), :], axis=1, keepdims=True)
        do8 = jnp.broadcast_to(do_row, (8, DH)).astype(BF)
        dq = _dot(do8, mhi[h], NT) + _dot(do8, mlo[h], NT)
        dq = (dq - dsum * hv[1, g, pl.ds(i, 1), :]) * SCALE
        dq_s[:, col] = jnp.where(row8 == b, dq, dq_s[:, col])
        row = pl.ds(st, 1)
        for rho in range(TPG):
            dp = _dot(do8, vbuf[(b * TPB + g * TPG + rho) % NV, st], NT)
            cols = slice(rho * QR, (rho + 1) * QR)
            coef[1, b, g, row, cols] = coef[0, b, g, row, cols] * ((dp[0:1] - dsum) * SCALE)

    def group(g, b):
        do_g = _dot(dh_s[...].astype(BF), wo_group(g), NT).astype(BF).astype(F32)
        row = lax.broadcasted_iota(jnp.int32, do_g.shape, 0)
        do_b = jnp.sum(jnp.where(row == b, do_g, 0.0), axis=0, keepdims=True)
        for i in range(HG):
            vec[0, b, g, i:i + 1, :] = do_b[:, i * DH:(i + 1) * DH]

        def dv_step(n, c):
            _, slot = fill_slot(0, b, g, n)
            issue_step(dv_hbm, b, g, n, slot)
            bwd_stream(b, g, n)
            return c

        def dk_step(n, c):
            j, slot = fill_slot(1, b, g, n)
            pl.when(jnp.logical_or(j < SPB - NDEF, j >= SPB))(lambda: issue_step(dk_hbm, b, g, n, slot))
            return c

        lax.fori_loop(0, NN_, dv_step, 0)
        lax.fori_loop(0, NN_, dk_step, 0)
        return b

    def batch(b, carry):
        lax.fori_loop(0, TPB, fwd_tile, b)

        @pl.when(b == 0)
        def _():
            v_load(TPB).fine(NBL - 1).start()
            k_early = k_load(TPB + 2)
            for j in range(NBL):
                if j >= AHEAD:
                    k_early.big(j).start(priority=1)
                k_early.fine(j).start(priority=1)

        middle(b)
        lax.fori_loop(0, NG, group, b)
        return carry

    lax.fori_loop(0, B, batch, 0)

    g8 = _rows8(g_v[...])
    dh = dh_s[...]
    outs = []

    def put(src, dst, i):
        cp = misc(src, dst, i)
        cp.start()
        outs.append(cp)

    def start_all(blocks):
        def body(j, c):
            blocks.big(j).start()
            return c
        lax.fori_loop(0, blocks.n, body, 0)

    dwq_w = _Blocks(wq_v, dwq_hbm, msem.at[4], None, (8, 8, 1024), 1, 0)
    dwo_w = _Blocks(wo_v, dwo_hbm, msem.at[5], None, (8, 16, D), 1, 0)
    dw1_w = _Blocks(w1_v, dw1_hbm, msem.at[6], None, (4, 8, F // 2), 1, 0)
    dw2_w = _Blocks(w2_v, dw2_hbm, msem.at[7], None, (4, 16, D), 1, 0)

    out8 = h1_s[...] + _dot(hid_s[...].astype(BF), _flat(w2_v[...]), NN) + b2_v[...].astype(F32).reshape(1, D)
    out_v[...] = out8[0:B].astype(BF)
    put(out_v, out_hbm, 0)
    db1_v[...] = jnp.sum(du_s[...], axis=0).astype(BF)
    db2_v[...] = jnp.sum(g8, axis=0).astype(BF)
    put(db1_v, db1_hbm, 2)
    put(db2_v, db2_hbm, 3)

    def dwo_group(g, c):
        wo_v[g] = _dot(o_s[:, group_cols(g)].astype(BF), dh_s[...].astype(BF), TN).astype(BF)
        return c

    lax.fori_loop(0, NG, dwo_group, 0)
    start_all(dwo_w)

    w1_v[...] = _dot(y2_s[...].astype(BF), du_s[...].astype(BF), TN).astype(BF).reshape(W1_SHAPE)
    w2_v[...] = _dot(hid_s[...].astype(BF), g8.astype(BF), TN).astype(BF).reshape(W2_SHAPE)

    def mlp_blocks(j, c):
        dw1_w.big(j).start()
        _start_if(j < dw2_w.n, dw2_w.big(jnp.minimum(j, dw2_w.n - 1)), 0)
        return c

    lax.fori_loop(0, dw1_w.n, mlp_blocks, 0)

    xn, r0 = _ln_fwd(_rows8(x_v[...]))

    def dwq_group(g, dxn):
        cols = group_cols(g)
        dq_g = dq_s[:, cols].astype(BF)
        dxn = dxn + _dot(dq_g, _flat(wq_v[:, :, cols]), NT)
        wq_v[:, :, cols] = _dot(xn.astype(BF), dq_g, TN).astype(BF).reshape(WQ_SHAPE[0], WQ_SHAPE[1], HG * DH)
        return dxn

    dxn = lax.fori_loop(0, NG, dwq_group, jnp.zeros((8, D), F32))
    dx_v[...] = (dh + _ln_bwd(dxn, xn, r0))[0:B].astype(BF)
    put(dx_v, dx_hbm, 1)
    start_all(dwq_w)

    for slot in range(NS):
        wait_slot(slot)
    for cp in outs:
        cp.wait()
    for blocks in (dwo_w, dw1_w, dw2_w, dwq_w):
        blocks.wait_big(0, blocks.n)


@jax.jit
def pallas_sequential_preLN__mha_block_cached__mixer_channel_mlp__decode_kernel(
    A_x: jax.Array,
    A_k_cache: jax.Array,
    A_v_cache: jax.Array,
    A_wq: jax.Array,
    A_wo: jax.Array,
    B_x: jax.Array,
    B_w1: jax.Array,
    B_b1: jax.Array,
    B_w2: jax.Array,
    B_b2: jax.Array,
    grad_out: jax.Array,
):
    del B_x
    any_spec = pl.BlockSpec(memory_space=pl.ANY)
    sds = jax.ShapeDtypeStruct
    out_shape = [
        sds((B, D), BF), sds((B, D), BF), sds(KV_SHAPE, BF), sds(KV_SHAPE, BF),
        sds(WQ_SHAPE, BF), sds(WO_SHAPE, BF),
        sds(W1_SHAPE, BF), sds((F,), BF), sds(W2_SHAPE, BF), sds((D,), BF),
    ]
    vm = pltpu.VMEM
    scratch = [
        vm((NK, G, QR, DH), BF), vm((NV, G, QR, DH), BF), vm((NS, R // C, G, C, DH), BF),
        vm(WQ_SHAPE, BF), vm(WO_SHAPE, BF), vm(W1_SHAPE, BF), vm(W2_SHAPE, BF),
        vm((B, D), BF), vm((B, D), BF), vm((F,), BF), vm((D,), BF),
        vm((2, B, NG, G, SR), F32), vm((2, B, NG, 8, DH), F32),
        vm((8, H * DH), F32), vm((2, NG, 8, DH), F32), vm((8, H * DH), F32),
        vm((H, DH, DH), BF), vm((H, DH, DH), BF), vm((8, S), F32), vm((8, S), F32),
        vm((G, 8, DH), F32), vm((HG, 8, DH), F32), vm((HG, 8, DH), F32),
        vm((HG, DH + 16, DH), F32), vm((HG, 16, DH), F32),
        vm((8, D), F32), vm((8, D), F32), vm((8, D), F32), vm((8, F), F32), vm((8, F), F32),
        vm((W2_SHAPE[0], 8, W2_SHAPE[1]), F32),
        vm((B, D), BF), vm((B, D), BF), vm((F,), BF), vm((D,), BF),
        pltpu.SemaphoreType.DMA((2 * NK,)), pltpu.SemaphoreType.DMA((2 * NK,)),
        pltpu.SemaphoreType.DMA((NS,)), pltpu.SemaphoreType.DMA((12,)),
    ]
    res = pl.pallas_call(
        _kernel,
        in_specs=[any_spec] * 10,
        out_specs=[any_spec] * 10,
        out_shape=out_shape,
        scratch_shapes=scratch,
        compiler_params=pltpu.CompilerParams(vmem_limit_bytes=120 * 1024 * 1024, disable_bounds_checks=NOBC,
                                             disable_semaphore_checks=NOBC),
    )(A_x.reshape(B, D), A_k_cache.reshape(KV_SHAPE), A_v_cache.reshape(KV_SHAPE),
      A_wq.reshape(WQ_SHAPE), A_wo.reshape(WO_SHAPE), B_w1.reshape(W1_SHAPE), B_b1,
      B_w2.reshape(W2_SHAPE), B_b2, grad_out.reshape(B, D))
    out, dx, dk, dv, dwq, dwo, dw1, db1, dw2, db2 = res
    return (out.reshape(B, 1, D), dx.reshape(B, 1, D), dk.reshape(B, H, S, DH), dv.reshape(B, H, S, DH),
            dwq.reshape(D, H * DH), dwo.reshape(H * DH, D), dw1.reshape(D, F), db1, dw2.reshape(F, D), db2)
```

```python
import jax
import jax.numpy as jnp
from jax import lax
import jax.experimental.pallas as pl
import jax.experimental.pallas.tpu as pltpu

BF = jnp.bfloat16
F32 = jnp.float32

B, H, S, DH, D, F = 2, 32, 8192, 128, 512, 1792
SCALE = DH ** -0.5
EPS = 1e-5

G = 8
SPH = 2
HG = G // SPH
SR = S // SPH
NG = H // HG
SHIFT = 1
GA = SHIFT * SPH
GB = G - GA
KV_SHAPE = (B, H * SPH, SR, DH)

QR = S // G
TPG = SR // QR
TPB = NG * TPG
T = B * TPB
NK = 3
NV = TPB + 1
BL = 64
FR = 8
BO = 8
NBL = QR // BL
LAG = 3
AHEAD = 4
MSUB = 512
NE = S // MSUB
FSKIP = (0, 8)
WOTICK = 6
assert NE == NBL and len(FSKIP) >= 1

R = 512
C = 64
CO = -24
NN_ = SR // R
SPB = 2 * NG * NN_
NS = 12
NLEFT = 1
NDEF = 8
CUTS = [0] + [c * C + CO for c in range(1, R // C)] + [R]
PIECES = [(lo, hi - lo) for lo, hi in zip(CUTS[:-1], CUTS[1:])]
assert NDEF <= NN_ and NN_ == G

WQ_SHAPE = (8, D // 8, H * DH)
WO_SHAPE = (NG, HG * DH, D)
W1_SHAPE = (4, D // 4, F)
W2_SHAPE = (4, F // 4, D)

NT = (((1,), (1,)), ((), ()))
NN = (((1,), (0,)), ((), ()))
TN = (((0,), (0,)), ((), ()))


def _dot(a, b, dims):
    return lax.dot_general(a, b, dims, preferred_element_type=F32)


def _ln_fwd(x):
    m = jnp.mean(x, axis=-1, keepdims=True)
    xc = x - m
    v = jnp.mean(xc * xc, axis=-1, keepdims=True)
    rstd = lax.rsqrt(v + EPS)
    return xc * rstd, rstd


def _ln_bwd(dy, y, rstd):
    m1 = jnp.mean(dy, axis=-1, keepdims=True)
    m2 = jnp.mean(dy * y, axis=-1, keepdims=True)
    return (dy - m1 - y * m2) * rstd


def _rows8(x2):
    return jnp.concatenate([x2.astype(F32), jnp.zeros((6, x2.shape[1]), F32)], axis=0)


def _flat(w3):
    return w3.reshape(w3.shape[0] * w3.shape[1], w3.shape[2])


def _aligned(x, n):
    return x if isinstance(x, int) else pl.multiple_of(x, n)


class _Blocks:
    def __init__(self, src, dst, sem, fsem, block, axis, fine_size):
        self.src, self.dst, self.sem, self.fsem = src, dst, sem, fsem
        self.block, self.axis, self.fine_size = block, axis, fine_size
        self.big_size = block[axis] - fine_size
        self.grid = [n // m for n, m in zip(dst.shape, block)]
        self.n = self.grid[0] * self.grid[1] * self.grid[2]

    def _part(self, j, offset, size, sem):
        at, inner = [], self.n
        for ax, align in enumerate((1, 8, DH)):
            outer, inner = inner, inner // self.grid[ax]
            pos = 0
            if self.grid[ax] > 1:
                pos = j if outer == self.n else j % outer
                pos = pos if inner == 1 else pos // inner
            lo = pos * self.block[ax] + (offset if ax == self.axis else 0)
            at.append(pl.ds(_aligned(lo, align), size if ax == self.axis else self.block[ax]))
        return pltpu.make_async_copy(self.src.at[tuple(at)], self.dst.at[tuple(at)], sem)

    def big(self, j):
        return self._part(j, 0, self.big_size, self.sem)

    def fine(self, j):
        return self._part(j, self.big_size, self.fine_size, self.fsem)

    def wait_big(self, lo, hi):
        for j in range(lo, hi):
            self.big(j).wait()

    def wait_fine(self):
        for j in range(self.n):
            self.fine(j).wait()


class _ShiftedBlocks(_Blocks):
    def big(self, j):
        if j == 0:
            return self._part(0, 0, self.big_size - BO, self.sem)
        return self._part(j, -BO, self.big_size, self.sem)

    def fine(self, j):
        return self._part(j, self.big_size - BO, self.fine_size + (BO if j == self.n - 1 else 0), self.fsem)


class _Pair:
    def __init__(self, first, second):
        self.copies = (first, second)

    def start(self, priority=0):
        for cp in self.copies:
            cp.start(priority=priority)

    def wait(self):
        for cp in self.copies:
            cp.wait()


class _BlockPairs(_Blocks):
    def __init__(self, first, second):
        self.parts, self.n = (first, second), first.n

    def big(self, j):
        return _Pair(*[p.big(j) for p in self.parts])

    def fine(self, j):
        return _Pair(*[p.fine(j) for p in self.parts])


def _head(g, i):
    return (g * HG + i + H - SHIFT) % H


def _segments(g):
    s0 = g * G - SHIFT * SPH
    return ((pl.ds((s0 + H * SPH) % (H * SPH), GA), pl.ds(0, GA)), (pl.ds(s0 + GA, GB), pl.ds(GA, GB)))


def _start_if(cond, copy, priority):
    pl.when(cond)(lambda: copy.start(priority=priority))


def _kernel(x_hbm, k_hbm, v_hbm, wq_hbm, wo_hbm, w1_hbm, b1_hbm, w2_hbm, b2_hbm, g_hbm,
            out_hbm, dx_hbm, dk_hbm, dv_hbm, dwq_hbm, dwo_hbm, dw1_hbm, db1_hbm, dw2_hbm, db2_hbm,
            kbuf, vbuf, stage, wq_v, wo_v, w1_v, w2_v, x_v, g_v, b1_v, b2_v,
            coef, vec, o_s, hv, dq_s, mhi, mlo, s_s, p_s, mx_s, m_s, l_s, macc, kacc,
            h1_s, dh_s, y2_s, du_s, hid_s, dhid_s,
            out_v, dx_v, db1_v, db2_v,
            ksem, vsem, wsem, msem):
    both = jnp.logical_and
    row8 = lax.broadcasted_iota(jnp.int32, (8, DH), 0)

    def tile_load(hbm, buf, nslot, sem, t, kind):
        rows = pl.ds(_aligned((t % TPG) * QR, QR), QR)
        return _BlockPairs(*[
            kind(hbm.at[t // TPB, far, rows], buf.at[t % nslot, near],
                 sem.at[t % NK], sem.at[NK + t % NK], (near.size, BL, DH), 1, FR)
            for far, near in _segments((t % TPB) // TPG)])

    def k_load(t, kind=_ShiftedBlocks):
        return tile_load(k_hbm, kbuf, NK, ksem, t, kind)

    def v_load(t, kind=_ShiftedBlocks):
        return tile_load(v_hbm, vbuf, NV, vsem, t, kind)

    def misc(src, dst, i):
        return pltpu.make_async_copy(src, dst, msem.at[i])

    def issue_step(dst, b, g, n, slot):
        def issue(segments):
            for lo, size in PIECES:
                rows = pl.ds(pl.multiple_of(n * R + lo, 8), size)
                for far, near in segments:
                    pltpu.make_async_copy(
                        stage.at[slot, near, pl.ds(lo, size)], dst.at[b, far, rows], wsem.at[slot]).start()

        if isinstance(g, int) and g > 0:
            issue([(pl.ds(g * G - SHIFT * SPH, G), pl.ds(0, G))])
        else:
            pl.when(g == 0)(lambda: issue(_segments(0)))
            pl.when(g > 0)(lambda: issue([(pl.ds(jnp.maximum(g * G - SHIFT * SPH, 0), G), pl.ds(0, G))]))

    def wait_slot(slot):
        pltpu.make_async_copy(stage.at[slot], stage.at[slot], wsem.at[slot]).wait()

    def wait_pieces(slot, lo, hi):
        for row, size in PIECES[lo:hi]:
            piece = stage.at[slot, :, pl.ds(row, size)]
            pltpu.make_async_copy(piece, piece, wsem.at[slot]).wait()

    def wo_group(g):
        cut = (HG - SHIFT) * DH
        return jnp.concatenate([wo_v[(g + NG - 1) % NG, cut:, :], wo_v[g, :cut, :]], axis=0)

    def group_cols(g):
        return pl.ds(_aligned(g * (HG * DH), HG * DH), HG * DH)

    def stream_scores(t, st):
        q_row = vec[1, t // TPB, (t % TPB) // TPG, pl.ds(st // SPH, 1), :]
        sc = _dot(jnp.broadcast_to(q_row, (8, DH)).astype(BF), kbuf[t % NK, st], NT)
        s_s[:, pl.ds(_aligned(st * QR, QR), QR)] = sc
        mx = sc[:, 0:DH]
        for tt in range(1, QR // DH):
            mx = jnp.maximum(mx, sc[:, tt * DH:(tt + 1) * DH])
        mx_s[st] = mx

    def add_attention(b, g):
        o_g = jnp.concatenate([jnp.where(row8 == b, hv[0, g, i:i + 1, :], 0.0) for i in range(HG)], axis=1)
        h1_s[...] += _dot(o_g.astype(BF), wo_group(g), NN)

    in_small = [misc(x_hbm, x_v, 0), misc(g_hbm, g_v, 1), misc(b1_hbm, b1_v, 2), misc(b2_hbm, b2_v, 3)]
    wq_l = _Blocks(wq_hbm, wq_v, msem.at[4], msem.at[8], (8, 8, 1024), 2, DH)
    wo_l = _Blocks(wo_hbm, wo_v, msem.at[5], msem.at[9], (4, 32, D), 1, 8)
    w1_l = _Blocks(w1_hbm, w1_v, msem.at[6], msem.at[10], (4, 8, F), 2, 2 * DH)
    w2_l = _Blocks(w2_hbm, w2_v, msem.at[7], msem.at[11], (4, 32, D), 1, 8)
    lag, depth = LAG + 1, LAG + 1 + AHEAD

    def paced(cur, nxt, count, work=None):
        def body(f, c):
            cur.big(f).wait()
            jf, jb = f + lag, f + depth
            _start_if(jf < cur.n, cur.fine(jnp.minimum(jf, cur.n - 1)), 0)
            _start_if(jf >= cur.n, nxt.fine(jnp.maximum(jf - cur.n, 0)), 0)
            _start_if(jb < cur.n, cur.big(jnp.minimum(jb, cur.n - 1)), 1)
            _start_if(jb >= cur.n, nxt.big(jnp.maximum(jb - cur.n, 0)), 1)
            if work is not None:
                pl.when(f % 2 == 0)(lambda: work(f // 2))
            return c
        lax.fori_loop(0, count, body, 0)

    for j in range(depth):
        wq_l.big(j).start(priority=1)
        if j == 0:
            for cp in in_small:
                cp.start()
        if j < lag:
            wq_l.fine(j).start()

    o_s[...] = jnp.zeros(o_s.shape, F32)
    dq_s[...] = jnp.zeros(dq_s.shape, F32)

    for cp in in_small:
        cp.wait()
    x8 = _rows8(x_v[...])
    h1_s[...] = x8
    y2_s[...] = _ln_fwd(x8)[0]

    def q_group(g):
        q_g = _dot(y2_s[...].astype(BF), _flat(wq_v[:, :, group_cols(g)]), NN).astype(BF).astype(F32)
        for bb in range(B):
            for i in range(HG):
                gg, ii = (g, i + SHIFT) if i + SHIFT < HG else ((g + 1) % NG, i + SHIFT - HG)
                vec[1, bb, gg, ii:ii + 1, :] = q_g[bb:bb + 1, i * DH:(i + 1) * DH]

    def dhid_part(j):
        @pl.when(j < W2_SHAPE[0])
        def _():
            jj = jnp.minimum(j, W2_SHAPE[0] - 1)
            dhid_s[jj] = _dot(_rows8(g_v[...]).astype(BF), w2_v[jj], NT)

    k0_l, k1_l, v0_l = k_load(0, _Blocks), k_load(1, _Blocks), v_load(0, _Blocks)
    paced(wq_l, k0_l, wq_l.n)
    wq_l.wait_fine()
    paced(k0_l, w2_l, NBL, q_group)
    k0_l.wait_fine()
    paced(w2_l, w1_l, w2_l.n)
    w2_l.wait_fine()
    paced(w1_l, wo_l, w1_l.n, lambda st: stream_scores(0, st))
    paced(wo_l, k1_l, wo_l.n, dhid_part)
    w1_l.wait_fine()
    paced(k1_l, v0_l, NBL)
    wo_l.wait_fine()
    k1_l.wait_fine()
    for f in range(NBL - lag):
        v0_l.big(f).wait()
        v0_l.fine(f + lag).start()
        (v0_l.big(f + depth) if f + depth < NBL else k_load(2).big(f + depth - NBL)).start(priority=1)

    def by_head(vals):
        res = vals[HG - 1]
        for i in range(HG - 2, -1, -1):
            res = jnp.where(row8 < (i + 1) * SPH, vals[i], res)
        return res

    def fwd_tile(tb, b):
        t = b * TPB + tb
        g, rho = tb // TPG, tb % TPG
        first, last = rho == 0, rho == TPG - 1
        ks, vs = t % NK, t % NV
        more1, more2, more3 = t + 1 < T, t + 2 < T, t + 3 < T
        tail = t == T - 2
        go2 = both(more2, t != TPB)
        t1 = jnp.minimum(t + 1, T - 1)
        v0, v1, v_end = v_load(t), v_load(t1), v_load(T - 1)
        k1, k2, k3 = k_load(t1), k_load(jnp.minimum(t + 2, T - 1)), k_load(jnp.minimum(t + 3, T - 1))
        last_slot = (SPB - NDEF - 1) % NS
        cc = S // NBL

        def starts(f):
            if f == 0:
                _start_if(both(more1, tb > 0), v0.fine(NBL - 1), 0)
            else:
                _start_if(go2, k2.fine(f - 1), 0)
                _start_if(tail, v_end.fine(f - 1), 0)
            if f + AHEAD < NBL:
                _start_if(go2, k2.big(f + AHEAD), 1)
                _start_if(tail, v_end.big(f + AHEAD), 1)
            elif f < NBL:
                _start_if(go2, v1.big(f + AHEAD - NBL), 1)

        pl.when(both(more1, t > 0))(lambda: v0.wait_big(0, NBL - lag))
        pl.when(more1)(v0.big(NBL - lag).wait)
        starts(0)

        alpha = []
        for i in range(HG):
            mx = mx_s[i * SPH]
            for z in range(1, SPH):
                mx = jnp.maximum(mx, mx_s[i * SPH + z])
            m_blk = jnp.broadcast_to(jnp.max(mx, axis=1, keepdims=True), (8, DH))
            m_old = jnp.where(first, m_blk, m_s[i])
            m_new = jnp.maximum(m_old, m_blk)
            m_s[i] = m_new
            alpha.append(jnp.exp((m_old - m_new) * SCALE))

        for f in range(NBL):
            cols = slice(f * cc, (f + 1) * cc)
            m = m_s[f // (NBL // HG)]
            p_s[:, cols] = jnp.exp((s_s[:, cols] - jnp.concatenate([m] * (cc // DH), axis=1)) * SCALE)
            if f == WOTICK:
                pl.when(both(first, g > 0))(lambda: add_attention(b, jnp.maximum(g - 1, 0)))
            if f < LAG:
                v0.big(NBL - LAG + f).wait()
            else:
                pl.when(more2)(k2.big(f - LAG).wait)
                pl.when(tail)(v_end.big(f - LAG).wait)
            starts(f + 1)

        pl.when(t > 0)(v0.wait_fine)
        pl.when(t == 0)(v0_l.wait_fine)

        @pl.when(both(more1, t > 0))
        def _():
            k1.wait_big(NBL - LAG, NBL)
            k1.wait_fine()

        @pl.when(tail)
        def _():
            def issue_deferred(n, c):
                issue_step(dk_hbm, 0, NG - 1, n, (SPB - NN_ + n) % NS)
                return c
            lax.fori_loop(NN_ - NDEF, NN_, issue_deferred, 0)

        @pl.when(t == TPB)
        def _():
            for j in range(SPB - NS, SPB - NDEF - 1):
                wait_slot(j % NS)
            wait_pieces(last_slot, 0, R // C - NLEFT)
            for j in range(AHEAD):
                v_load(TPB + 1).big(j).start(priority=1)

        fin = []
        for i in range(HG):
            acc = jnp.where(first, 0.0, macc[i] * alpha[i][0:1])
            kb = jnp.where(first, 0.0, kacc[i] * alpha[i][0:1])
            tot = jnp.where(first, 0.0, l_s[i] * alpha[i])
            for u in range(i * NE // HG, (i + 1) * NE // HG):
                if u not in FSKIP:
                    _start_if(more2, v1.fine(u - sum(x < u for x in FSKIP)), 0)
                if u + AHEAD < NBL:
                    _start_if(more2, v1.big(u + AHEAD), 1)
                else:
                    _start_if(t == T - 3, v_end.big(u + AHEAD - NBL), 1)
                r = u * MSUB
                st, r0 = r // QR, r % QR
                kc = kbuf[ks, st, r0:r0 + MSUB, :]
                p8 = p_s[:, r:r + MSUB]
                for tt in range(MSUB // DH):
                    tot = tot + p8[:, tt * DH:(tt + 1) * DH]
                p_hi = p8.astype(BF).astype(F32)
                p16 = jnp.concatenate([p_hi, p8 - p_hi], axis=0)
                a = kc.astype(F32).T * p_s[0:1, r:r + MSUB]
                lhs = jnp.concatenate([a, p16], axis=0).astype(BF)
                acc = acc + _dot(lhs, vbuf[vs, st, r0:r0 + MSUB, :], NN)
                kb = kb + _dot(p16.astype(BF), kc, NN)
                if u == NE - 1:
                    for j in range(NE - len(FSKIP), NBL - 1):
                        _start_if(more2, v1.fine(j), 0)
                    for j in range(AHEAD):
                        _start_if(more3, k3.big(j), 1)
                if u % (NE // G) == NE // G - 1:
                    stream_scores(t1, u // (NE // G))
            macc[i] = acc
            kacc[i] = kb
            l_s[i] = tot
            inv = jnp.broadcast_to(1.0 / jnp.sum(tot, axis=1, keepdims=True), (8, DH))
            mt = acc[0:DH] * inv[0:1]
            mt_hi = mt.astype(BF)
            mhi[g * HG + i] = mt_hi
            mlo[g * HG + i] = (mt - mt_hi.astype(F32)).astype(BF)
            o8 = (acc[DH:DH + 8] + acc[DH + 8:DH + 16]) * inv
            hv[0, g, i:i + 1, :] = o8[0:1]
            hv[1, g, i:i + 1, :] = (kb[0:1] + kb[8:9]) * inv[0:1]
            col = pl.ds(pl.multiple_of(_head(g, i) * DH, DH), DH)
            o_s[:, col] = jnp.where(row8 == b, o8, o_s[:, col])
            fin.append(jnp.where(last, inv, 1.0))

        f_new = by_head(fin)
        f_old = by_head(alpha) * f_new
        for tt in range((SR - QR) // DH):
            cols = slice(tt * DH, (tt + 1) * DH)
            coef[0, b, g, :, cols] = jnp.where(tt * DH < rho * QR, coef[0, b, g, :, cols] * f_old, 0.0)
        for tt in range(QR // DH):
            blk = p_s[:, (G - 1) * QR + tt * DH:(G - 1) * QR + (tt + 1) * DH]
            for st in range(G - 2, -1, -1):
                blk = jnp.where(row8 == st, p_s[:, st * QR + tt * DH:st * QR + (tt + 1) * DH], blk)
            coef[0, b, g, :, pl.ds(pl.multiple_of(rho * QR + tt * DH, DH), DH)] = blk * f_new

        pl.when(t == TPB)(lambda: wait_pieces(last_slot, R // C - NLEFT, R // C))
        return b

    def middle(b):
        add_attention(b, NG - 1)
        y1, r1 = _ln_fwd(h1_s[...])
        y2, r2 = _ln_fwd(y1)
        u = _dot(y2.astype(BF), _flat(w1_v[...]), NN) + b1_v[...].astype(F32).reshape(1, F)
        c0 = (2.0 / jnp.pi) ** 0.5
        th = jnp.tanh(c0 * (u + 0.044715 * (u * u * u)))
        dgelu = 0.5 * (1.0 + th) + 0.5 * u * (1.0 - th * th) * (c0 * (1.0 + 3 * 0.044715 * (u * u)))
        du = jnp.concatenate([dhid_s[j] for j in range(W2_SHAPE[0])], axis=1) * dgelu
        dy2 = _dot(du.astype(BF), _flat(w1_v[...]), NT)
        dh_s[...] = _rows8(g_v[...]) + _ln_bwd(_ln_bwd(dy2, y2, r2), y1, r1)
        y2_s[...] = y2
        du_s[...] = du
        hid_s[...] = 0.5 * u * (1.0 + th)

    eye = (lax.broadcasted_iota(jnp.int32, (DH, DH), 0) == lax.broadcasted_iota(jnp.int32, (DH, DH), 1))

    def fill_slot(kind, b, g, n):
        j = b * SPB + (2 * g + kind) * NN_ + n
        slot = j % NS
        drained = both(j >= SPB, j < SPB + NS - NDEF)
        pl.when(both(j >= NS, jnp.logical_not(drained)))(lambda: wait_slot(slot))

        for i in range(HG):
            w = jnp.broadcast_to(vec[kind, b, g, i:i + 1, :], (DH, DH)).astype(BF)
            tiles = []
            for z in range(SPH):
                for tt in range(R // DH):
                    r = pl.multiple_of(n * R + tt * DH, DH)
                    cf = coef[kind, b, g, pl.ds(i * SPH + z, 1), pl.ds(r, DH)]
                    tiles.append(jnp.where(eye, cf, 0.0).astype(BF))
            res = _dot(jnp.concatenate(tiles, axis=0), w, NN).astype(BF)
            for z in range(SPH):
                stage[slot, i * SPH + z] = res[z * R:(z + 1) * R]
        return j, slot

    def bwd_stream(b, g, st):
        i = st // SPH
        h = g * HG + i
        col = pl.ds(pl.multiple_of(_head(g, i) * DH, DH), DH)
        do_row = vec[0, b, g, pl.ds(i, 1), :]
        dsum = jnp.sum(do_row * hv[0, g, pl.ds(i, 1), :], axis=1, keepdims=True)
        do8 = jnp.broadcast_to(do_row, (8, DH)).astype(BF)
        dq = _dot(do8, mhi[h], NT) + _dot(do8, mlo[h], NT)
        dq = (dq - dsum * hv[1, g, pl.ds(i, 1), :]) * SCALE
        dq_s[:, col] = jnp.where(row8 == b, dq, dq_s[:, col])
        row = pl.ds(st, 1)
        for rho in range(TPG):
            dp = _dot(do8, vbuf[(b * TPB + g * TPG + rho) % NV, st], NT)
            cols = slice(rho * QR, (rho + 1) * QR)
            coef[1, b, g, row, cols] = coef[0, b, g, row, cols] * ((dp[0:1] - dsum) * SCALE)

    def group(g, b):
        do_g = _dot(dh_s[...].astype(BF), wo_group(g), NT).astype(BF).astype(F32)
        row = lax.broadcasted_iota(jnp.int32, do_g.shape, 0)
        do_b = jnp.sum(jnp.where(row == b, do_g, 0.0), axis=0, keepdims=True)
        for i in range(HG):
            vec[0, b, g, i:i + 1, :] = do_b[:, i * DH:(i + 1) * DH]

        def dv_step(n, c):
            _, slot = fill_slot(0, b, g, n)
            issue_step(dv_hbm, b, g, n, slot)
            bwd_stream(b, g, n)
            return c

        def dk_step(n, c):
            j, slot = fill_slot(1, b, g, n)
            pl.when(jnp.logical_or(j < SPB - NDEF, j >= SPB))(lambda: issue_step(dk_hbm, b, g, n, slot))
            return c

        lax.fori_loop(0, NN_, dv_step, 0)
        lax.fori_loop(0, NN_, dk_step, 0)
        return b

    def batch(b, carry):
        lax.fori_loop(0, TPB, fwd_tile, b)

        @pl.when(b == 0)
        def _():
            v_load(TPB).fine(NBL - 1).start()
            k_early = k_load(TPB + 2)
            for j in range(NBL):
                if j >= AHEAD:
                    k_early.big(j).start(priority=1)
                k_early.fine(j).start(priority=1)

        middle(b)
        lax.fori_loop(0, NG, group, b)
        return carry

    lax.fori_loop(0, B, batch, 0)

    g8 = _rows8(g_v[...])
    dh = dh_s[...]
    outs = []

    def put(src, dst, i):
        cp = misc(src, dst, i)
        cp.start()
        outs.append(cp)

    def start_all(blocks):
        def body(j, c):
            blocks.big(j).start()
            return c
        lax.fori_loop(0, blocks.n, body, 0)

    dwq_w = _Blocks(wq_v, dwq_hbm, msem.at[4], None, (8, 8, 1024), 1, 0)
    dwo_w = _Blocks(wo_v, dwo_hbm, msem.at[5], None, (8, 16, D), 1, 0)
    dw1_w = _Blocks(w1_v, dw1_hbm, msem.at[6], None, (4, 8, F // 2), 1, 0)
    dw2_w = _Blocks(w2_v, dw2_hbm, msem.at[7], None, (4, 16, D), 1, 0)

    out8 = h1_s[...] + _dot(hid_s[...].astype(BF), _flat(w2_v[...]), NN) + b2_v[...].astype(F32).reshape(1, D)
    out_v[...] = out8[0:B].astype(BF)
    put(out_v, out_hbm, 0)
    db1_v[...] = jnp.sum(du_s[...], axis=0).astype(BF)
    db2_v[...] = jnp.sum(g8, axis=0).astype(BF)
    put(db1_v, db1_hbm, 2)
    put(db2_v, db2_hbm, 3)

    def dwo_group(g, c):
        wo_v[g] = _dot(o_s[:, group_cols(g)].astype(BF), dh_s[...].astype(BF), TN).astype(BF)
        return c

    lax.fori_loop(0, NG, dwo_group, 0)
    start_all(dwo_w)

    w1_v[...] = _dot(y2_s[...].astype(BF), du_s[...].astype(BF), TN).astype(BF).reshape(W1_SHAPE)
    w2_v[...] = _dot(hid_s[...].astype(BF), g8.astype(BF), TN).astype(BF).reshape(W2_SHAPE)

    def mlp_blocks(j, c):
        dw1_w.big(j).start()
        _start_if(j < dw2_w.n, dw2_w.big(jnp.minimum(j, dw2_w.n - 1)), 0)
        return c

    lax.fori_loop(0, dw1_w.n, mlp_blocks, 0)

    xn, r0 = _ln_fwd(_rows8(x_v[...]))

    def dwq_group(g, dxn):
        cols = group_cols(g)
        dq_g = dq_s[:, cols].astype(BF)
        dxn = dxn + _dot(dq_g, _flat(wq_v[:, :, cols]), NT)
        wq_v[:, :, cols] = _dot(xn.astype(BF), dq_g, TN).astype(BF).reshape(WQ_SHAPE[0], WQ_SHAPE[1], HG * DH)
        return dxn

    dxn = lax.fori_loop(0, NG, dwq_group, jnp.zeros((8, D), F32))
    dx_v[...] = (dh + _ln_bwd(dxn, xn, r0))[0:B].astype(BF)
    put(dx_v, dx_hbm, 1)
    start_all(dwq_w)

    for slot in range(NS):
        wait_slot(slot)
    for cp in outs:
        cp.wait()
    for blocks in (dwo_w, dw1_w, dw2_w, dwq_w):
        blocks.wait_big(0, blocks.n)


@jax.jit
def pallas_sequential_preLN__mha_block_cached__mixer_channel_mlp__decode_kernel(
    A_x: jax.Array,
    A_k_cache: jax.Array,
    A_v_cache: jax.Array,
    A_wq: jax.Array,
    A_wo: jax.Array,
    B_x: jax.Array,
    B_w1: jax.Array,
    B_b1: jax.Array,
    B_w2: jax.Array,
    B_b2: jax.Array,
    grad_out: jax.Array,
):
    del B_x
    any_spec = pl.BlockSpec(memory_space=pl.ANY)
    sds = jax.ShapeDtypeStruct
    out_shape = [
        sds((B, D), BF), sds((B, D), BF), sds(KV_SHAPE, BF), sds(KV_SHAPE, BF),
        sds(WQ_SHAPE, BF), sds(WO_SHAPE, BF),
        sds(W1_SHAPE, BF), sds((F,), BF), sds(W2_SHAPE, BF), sds((D,), BF),
    ]
    vm = pltpu.VMEM
    scratch = [
        vm((NK, G, QR, DH), BF), vm((NV, G, QR, DH), BF), vm((NS, G, R, DH), BF),
        vm(WQ_SHAPE, BF), vm(WO_SHAPE, BF), vm(W1_SHAPE, BF), vm(W2_SHAPE, BF),
        vm((B, D), BF), vm((B, D), BF), vm((F,), BF), vm((D,), BF),
        vm((2, B, NG, G, SR), F32), vm((2, B, NG, 8, DH), F32),
        vm((8, H * DH), F32), vm((2, NG, 8, DH), F32), vm((8, H * DH), F32),
        vm((H, DH, DH), BF), vm((H, DH, DH), BF), vm((8, S), F32), vm((8, S), F32),
        vm((G, 8, DH), F32), vm((HG, 8, DH), F32), vm((HG, 8, DH), F32),
        vm((HG, DH + 16, DH), F32), vm((HG, 16, DH), F32),
        vm((8, D), F32), vm((8, D), F32), vm((8, D), F32), vm((8, F), F32), vm((8, F), F32),
        vm((W2_SHAPE[0], 8, W2_SHAPE[1]), F32),
        vm((B, D), BF), vm((B, D), BF), vm((F,), BF), vm((D,), BF),
        pltpu.SemaphoreType.DMA((2 * NK,)), pltpu.SemaphoreType.DMA((2 * NK,)),
        pltpu.SemaphoreType.DMA((NS,)), pltpu.SemaphoreType.DMA((12,)),
    ]
    res = pl.pallas_call(
        _kernel,
        in_specs=[any_spec] * 10,
        out_specs=[any_spec] * 10,
        out_shape=out_shape,
        scratch_shapes=scratch,
        compiler_params=pltpu.CompilerParams(
            vmem_limit_bytes=120 * 1024 * 1024, disable_bounds_checks=True, disable_semaphore_checks=True),
    )(A_x.reshape(B, D), A_k_cache.reshape(KV_SHAPE), A_v_cache.reshape(KV_SHAPE),
      A_wq.reshape(WQ_SHAPE), A_wo.reshape(WO_SHAPE), B_w1.reshape(W1_SHAPE), B_b1,
      B_w2.reshape(W2_SHAPE), B_b2, grad_out.reshape(B, D))
    out, dx, dk, dv, dwq, dwo, dw1, db1, dw2, db2 = res
    return (out.reshape(B, 1, D), dx.reshape(B, 1, D), dk.reshape(B, H, S, DH), dv.reshape(B, H, S, DH),
            dwq.reshape(D, H * DH), dwo.reshape(H * DH, D), dw1.reshape(D, F), db1, dw2.reshape(F, D), db2)
```

```python
import dataclasses

import jax
import jax.numpy as jnp
from jax import lax
import jax.experimental.pallas as pl
import jax.experimental.pallas.tpu as pltpu

BF = jnp.bfloat16
F32 = jnp.float32

B, H, S, DH, D, F = 2, 32, 8192, 128, 512, 1792
SCALE = DH ** -0.5
EPS = 1e-5

G = 8
SPH = 2
HG = G // SPH
SR = S // SPH
NG = H // HG
SHIFT = 1
GA = SHIFT * SPH
GB = G - GA
KV_SHAPE = (B, H * SPH, SR, DH)

QR = S // G
TPG = SR // QR
TPB = NG * TPG
T = B * TPB
NK = 3
NV = TPB + 1
BL = 64
FR = 8
BO = 8
NBL = QR // BL
LAG = 3
AHEAD = 4
MSUB = 512
NE = S // MSUB
FSKIP = (0, 8)
WOTICK = 6
assert NE == NBL and len(FSKIP) >= 1

R = 512
C = 64
CO = -24
NN_ = SR // R
SPB = 2 * NG * NN_
NS = 12
NLEFT = 1
NDEF = 8
CUTS = [0] + [c * C + CO for c in range(1, R // C)] + [R]
PIECES = [(lo, hi - lo) for lo, hi in zip(CUTS[:-1], CUTS[1:])]
assert NDEF <= NN_ and NN_ == G

WQ_SHAPE = (8, D // 8, H * DH)
WO_SHAPE = (NG, HG * DH, D)
W1_SHAPE = (4, D // 4, F)
W2_SHAPE = (4, F // 4, D)

NT = (((1,), (1,)), ((), ()))
NN = (((1,), (0,)), ((), ()))
TN = (((0,), (0,)), ((), ()))


def _dot(a, b, dims):
    return lax.dot_general(a, b, dims, preferred_element_type=F32)


def _ln_fwd(x):
    m = jnp.mean(x, axis=-1, keepdims=True)
    xc = x - m
    v = jnp.mean(xc * xc, axis=-1, keepdims=True)
    rstd = lax.rsqrt(v + EPS)
    return xc * rstd, rstd


def _ln_bwd(dy, y, rstd):
    m1 = jnp.mean(dy, axis=-1, keepdims=True)
    m2 = jnp.mean(dy * y, axis=-1, keepdims=True)
    return (dy - m1 - y * m2) * rstd


def _rows8(x2):
    return jnp.concatenate([x2.astype(F32), jnp.zeros((6, x2.shape[1]), F32)], axis=0)


def _flat(w3):
    return w3.reshape(w3.shape[0] * w3.shape[1], w3.shape[2])


def _aligned(x, n):
    return x if isinstance(x, int) else pl.multiple_of(x, n)


class _Blocks:
    def __init__(self, src, dst, sem, fsem, block, axis, fine_size):
        self.src, self.dst, self.sem, self.fsem = src, dst, sem, fsem
        self.block, self.axis, self.fine_size = block, axis, fine_size
        self.big_size = block[axis] - fine_size
        self.grid = [n // m for n, m in zip(dst.shape, block)]
        self.n = self.grid[0] * self.grid[1] * self.grid[2]

    def _part(self, j, offset, size, sem):
        at, inner = [], self.n
        for ax, align in enumerate((1, 8, DH)):
            outer, inner = inner, inner // self.grid[ax]
            pos = 0
            if self.grid[ax] > 1:
                pos = j if outer == self.n else j % outer
                pos = pos if inner == 1 else pos // inner
            lo = pos * self.block[ax] + (offset if ax == self.axis else 0)
            at.append(pl.ds(_aligned(lo, align), size if ax == self.axis else self.block[ax]))
        return pltpu.make_async_copy(self.src.at[tuple(at)], self.dst.at[tuple(at)], sem)

    def big(self, j):
        return self._part(j, 0, self.big_size, self.sem)

    def fine(self, j):
        return self._part(j, self.big_size, self.fine_size, self.fsem)

    def wait_big(self, lo, hi):
        for j in range(lo, hi):
            self.big(j).wait()

    def wait_fine(self):
        for j in range(self.n):
            self.fine(j).wait()


class _ShiftedBlocks(_Blocks):
    def big(self, j):
        if j == 0:
            return self._part(0, 0, self.big_size - BO, self.sem)
        return self._part(j, -BO, self.big_size, self.sem)

    def fine(self, j):
        return self._part(j, self.big_size - BO, self.fine_size + (BO if j == self.n - 1 else 0), self.fsem)


class _Pair:
    def __init__(self, first, second):
        self.copies = (first, second)

    def start(self, priority=0):
        for cp in self.copies:
            cp.start(priority=priority)

    def wait(self):
        for cp in self.copies:
            cp.wait()


class _BlockPairs(_Blocks):
    def __init__(self, first, second):
        self.parts, self.n = (first, second), first.n

    def big(self, j):
        return _Pair(*[p.big(j) for p in self.parts])

    def fine(self, j):
        return _Pair(*[p.fine(j) for p in self.parts])


def _head(g, i):
    return (g * HG + i + H - SHIFT) % H


def _segments(g):
    s0 = g * G - SHIFT * SPH
    return ((pl.ds((s0 + H * SPH) % (H * SPH), GA), pl.ds(0, GA)), (pl.ds(s0 + GA, GB), pl.ds(GA, GB)))


def _start_if(cond, copy, priority):
    pl.when(cond)(lambda: copy.start(priority=priority))


def _kernel(x_hbm, k_hbm, v_hbm, wq_hbm, wo_hbm, w1_hbm, b1_hbm, w2_hbm, b2_hbm, g_hbm,
            out_hbm, dx_hbm, dk_hbm, dv_hbm, dwq_hbm, dwo_hbm, dw1_hbm, db1_hbm, dw2_hbm, db2_hbm,
            kbuf, vbuf, stage, wq_v, wo_v, w1_v, w2_v, x_v, g_v, b1_v, b2_v,
            coef, vec, o_s, hv, dq_s, mhi, mlo, s_s, p_s, mx_s, m_s, l_s, macc, kacc,
            h1_s, dh_s, y2_s, du_s, hid_s, dhid_s,
            out_v, dx_v, db1_v, db2_v,
            ksem, vsem, wsem, msem):
    both = jnp.logical_and
    row8 = lax.broadcasted_iota(jnp.int32, (8, DH), 0)

    def tile_load(hbm, buf, nslot, sem, t, kind):
        rows = pl.ds(_aligned((t % TPG) * QR, QR), QR)
        return _BlockPairs(*[
            kind(hbm.at[t // TPB, far, rows], buf.at[t % nslot, near],
                 sem.at[t % NK], sem.at[NK + t % NK], (near.size, BL, DH), 1, FR)
            for far, near in _segments((t % TPB) // TPG)])

    def k_load(t, kind=_ShiftedBlocks):
        return tile_load(k_hbm, kbuf, NK, ksem, t, kind)

    def v_load(t, kind=_ShiftedBlocks):
        return tile_load(v_hbm, vbuf, NV, vsem, t, kind)

    def misc(src, dst, i):
        return pltpu.make_async_copy(src, dst, msem.at[i])

    def issue_step(dst, b, g, n, slot):
        def issue(segments):
            for lo, size in PIECES:
                rows = pl.ds(pl.multiple_of(n * R + lo, 8), size)
                for far, near in segments:
                    pltpu.make_async_copy(
                        stage.at[slot, near, pl.ds(lo, size)], dst.at[b, far, rows], wsem.at[slot]).start()

        if isinstance(g, int) and g > 0:
            issue([(pl.ds(g * G - SHIFT * SPH, G), pl.ds(0, G))])
        else:
            pl.when(g == 0)(lambda: issue(_segments(0)))
            pl.when(g > 0)(lambda: issue([(pl.ds(jnp.maximum(g * G - SHIFT * SPH, 0), G), pl.ds(0, G))]))

    def wait_slot(slot):
        pltpu.make_async_copy(stage.at[slot], stage.at[slot], wsem.at[slot]).wait()

    def wait_pieces(slot, lo, hi):
        for row, size in PIECES[lo:hi]:
            piece = stage.at[slot, :, pl.ds(row, size)]
            pltpu.make_async_copy(piece, piece, wsem.at[slot]).wait()

    def wo_group(g):
        cut = (HG - SHIFT) * DH
        return jnp.concatenate([wo_v[(g + NG - 1) % NG, cut:, :], wo_v[g, :cut, :]], axis=0)

    def group_cols(g):
        return pl.ds(_aligned(g * (HG * DH), HG * DH), HG * DH)

    def stream_scores(t, st):
        q_row = vec[1, t // TPB, (t % TPB) // TPG, pl.ds(st // SPH, 1), :]
        sc = _dot(jnp.broadcast_to(q_row, (8, DH)).astype(BF), kbuf[t % NK, st], NT)
        s_s[:, pl.ds(_aligned(st * QR, QR), QR)] = sc
        mx = sc[:, 0:DH]
        for tt in range(1, QR // DH):
            mx = jnp.maximum(mx, sc[:, tt * DH:(tt + 1) * DH])
        mx_s[st] = mx

    def add_attention(b, g):
        o_g = jnp.concatenate([jnp.where(row8 == b, hv[0, g, i:i + 1, :], 0.0) for i in range(HG)], axis=1)
        h1_s[...] += _dot(o_g.astype(BF), wo_group(g), NN)

    in_small = [misc(x_hbm, x_v, 0), misc(g_hbm, g_v, 1), misc(b1_hbm, b1_v, 2), misc(b2_hbm, b2_v, 3)]
    wq_l = _Blocks(wq_hbm, wq_v, msem.at[4], msem.at[8], (8, 8, 1024), 2, DH)
    wo_l = _Blocks(wo_hbm, wo_v, msem.at[5], msem.at[9], (4, 32, D), 1, 8)
    w1_l = _Blocks(w1_hbm, w1_v, msem.at[6], msem.at[10], (4, 8, F), 2, 2 * DH)
    w2_l = _Blocks(w2_hbm, w2_v, msem.at[7], msem.at[11], (4, 32, D), 1, 8)
    lag, depth = LAG + 1, LAG + 1 + AHEAD

    def paced(cur, nxt, count, work=None):
        def body(f, c):
            cur.big(f).wait()
            jf, jb = f + lag, f + depth
            _start_if(jf < cur.n, cur.fine(jnp.minimum(jf, cur.n - 1)), 0)
            _start_if(jf >= cur.n, nxt.fine(jnp.maximum(jf - cur.n, 0)), 0)
            _start_if(jb < cur.n, cur.big(jnp.minimum(jb, cur.n - 1)), 1)
            _start_if(jb >= cur.n, nxt.big(jnp.maximum(jb - cur.n, 0)), 1)
            if work is not None:
                pl.when(f % 2 == 0)(lambda: work(f // 2))
            return c
        lax.fori_loop(0, count, body, 0)

    for j in range(depth):
        wq_l.big(j).start(priority=1)
        if j == 0:
            for cp in in_small:
                cp.start()
        if j < lag:
            wq_l.fine(j).start()

    o_s[...] = jnp.zeros(o_s.shape, F32)
    dq_s[...] = jnp.zeros(dq_s.shape, F32)

    for cp in in_small:
        cp.wait()
    x8 = _rows8(x_v[...])
    h1_s[...] = x8
    y2_s[...] = _ln_fwd(x8)[0]

    def clear_probs(j):
        coef[0, j // NG, j % NG] = jnp.zeros((G, SR), F32)

    def q_group(g):
        q_g = _dot(y2_s[...].astype(BF), _flat(wq_v[:, :, group_cols(g)]), NN).astype(BF).astype(F32)
        for bb in range(B):
            for i in range(HG):
                gg, ii = (g, i + SHIFT) if i + SHIFT < HG else ((g + 1) % NG, i + SHIFT - HG)
                vec[1, bb, gg, ii:ii + 1, :] = q_g[bb:bb + 1, i * DH:(i + 1) * DH]

    def dhid_part(j):
        @pl.when(j < W2_SHAPE[0])
        def _():
            jj = jnp.minimum(j, W2_SHAPE[0] - 1)
            dhid_s[jj] = _dot(_rows8(g_v[...]).astype(BF), w2_v[jj], NT)

    k0_l, k1_l, v0_l = k_load(0, _Blocks), k_load(1, _Blocks), v_load(0, _Blocks)
    assert wq_l.n == 2 * B * NG and NBL == 2 * NG and w1_l.n == 2 * G
    paced(wq_l, k0_l, wq_l.n, clear_probs)
    wq_l.wait_fine()
    paced(k0_l, w2_l, NBL, q_group)
    k0_l.wait_fine()
    paced(w2_l, w1_l, w2_l.n)
    w2_l.wait_fine()
    paced(w1_l, wo_l, w1_l.n, lambda st: stream_scores(0, st))
    paced(wo_l, k1_l, wo_l.n, dhid_part)
    w1_l.wait_fine()
    paced(k1_l, v0_l, NBL)
    wo_l.wait_fine()
    k1_l.wait_fine()
    for f in range(NBL - lag):
        v0_l.big(f).wait()
        v0_l.fine(f + lag).start()
        (v0_l.big(f + depth) if f + depth < NBL else k_load(2).big(f + depth - NBL)).start(priority=1)

    def by_head(vals):
        res = vals[HG - 1]
        for i in range(HG - 2, -1, -1):
            res = jnp.where(row8 < (i + 1) * SPH, vals[i], res)
        return res

    def fwd_tile(tb, b):
        t = b * TPB + tb
        g, rho = tb // TPG, tb % TPG
        first, last = rho == 0, rho == TPG - 1
        ks, vs = t % NK, t % NV
        more1, more2, more3 = t + 1 < T, t + 2 < T, t + 3 < T
        tail = t == T - 2
        go2 = both(more2, t != TPB)
        t1 = jnp.minimum(t + 1, T - 1)
        v0, v1, v_end = v_load(t), v_load(t1), v_load(T - 1)
        k1, k2, k3 = k_load(t1), k_load(jnp.minimum(t + 2, T - 1)), k_load(jnp.minimum(t + 3, T - 1))
        last_slot = (SPB - NDEF - 1) % NS
        cc = S // NBL

        def starts(f):
            if f == 0:
                _start_if(both(more1, tb > 0), v0.fine(NBL - 1), 0)
            else:
                _start_if(go2, k2.fine(f - 1), 0)
                _start_if(tail, v_end.fine(f - 1), 0)
            if f + AHEAD < NBL:
                _start_if(go2, k2.big(f + AHEAD), 1)
                _start_if(tail, v_end.big(f + AHEAD), 1)
            elif f < NBL:
                _start_if(go2, v1.big(f + AHEAD - NBL), 1)

        pl.when(both(more1, t > 0))(lambda: v0.wait_big(0, NBL - lag))
        pl.when(more1)(v0.big(NBL - lag).wait)
        starts(0)

        alpha = []
        for i in range(HG):
            mx = mx_s[i * SPH]
            for z in range(1, SPH):
                mx = jnp.maximum(mx, mx_s[i * SPH + z])
            m_blk = jnp.broadcast_to(jnp.max(mx, axis=1, keepdims=True), (8, DH))
            m_old = jnp.where(first, m_blk, m_s[i])
            m_new = jnp.maximum(m_old, m_blk)
            m_s[i] = m_new
            alpha.append(jnp.exp((m_old - m_new) * SCALE))

        for f in range(NBL):
            cols = slice(f * cc, (f + 1) * cc)
            m = m_s[f // (NBL // HG)]
            p_s[:, cols] = jnp.exp((s_s[:, cols] - jnp.concatenate([m] * (cc // DH), axis=1)) * SCALE)
            if f == WOTICK:
                pl.when(both(first, g > 0))(lambda: add_attention(b, jnp.maximum(g - 1, 0)))
            if f < LAG:
                v0.big(NBL - LAG + f).wait()
            else:
                pl.when(more2)(k2.big(f - LAG).wait)
                pl.when(tail)(v_end.big(f - LAG).wait)
            starts(f + 1)

        pl.when(t > 0)(v0.wait_fine)
        pl.when(t == 0)(v0_l.wait_fine)

        @pl.when(both(more1, t > 0))
        def _():
            k1.wait_big(NBL - LAG, NBL)
            k1.wait_fine()

        @pl.when(tail)
        def _():
            def issue_deferred(n, c):
                issue_step(dk_hbm, 0, NG - 1, n, (SPB - NN_ + n) % NS)
                return c
            lax.fori_loop(NN_ - NDEF, NN_, issue_deferred, 0)

        @pl.when(t == TPB)
        def _():
            for j in range(SPB - NS, SPB - NDEF - 1):
                wait_slot(j % NS)
            wait_pieces(last_slot, 0, R // C - NLEFT)
            for j in range(AHEAD):
                v_load(TPB + 1).big(j).start(priority=1)

        fin = []
        for i in range(HG):
            acc = jnp.where(first, 0.0, macc[i] * alpha[i][0:1])
            kb = jnp.where(first, 0.0, kacc[i] * alpha[i][0:1])
            tot = jnp.where(first, 0.0, l_s[i] * alpha[i])
            for u in range(i * NE // HG, (i + 1) * NE // HG):
                if u not in FSKIP:
                    _start_if(more2, v1.fine(u - sum(x < u for x in FSKIP)), 0)
                if u + AHEAD < NBL:
                    _start_if(more2, v1.big(u + AHEAD), 1)
                else:
                    _start_if(t == T - 3, v_end.big(u + AHEAD - NBL), 1)
                r = u * MSUB
                st, r0 = r // QR, r % QR
                kc = kbuf[ks, st, r0:r0 + MSUB, :]
                p8 = p_s[:, r:r + MSUB]
                for tt in range(MSUB // DH):
                    tot = tot + p8[:, tt * DH:(tt + 1) * DH]
                p_hi = p8.astype(BF).astype(F32)
                p16 = jnp.concatenate([p_hi, p8 - p_hi], axis=0)
                a = kc.astype(F32).T * p_s[0:1, r:r + MSUB]
                lhs = jnp.concatenate([a, p16], axis=0).astype(BF)
                acc = acc + _dot(lhs, vbuf[vs, st, r0:r0 + MSUB, :], NN)
                kb = kb + _dot(p16.astype(BF), kc, NN)
                if u == NE - 1:
                    for j in range(NE - len(FSKIP), NBL - 1):
                        _start_if(more2, v1.fine(j), 0)
                    for j in range(AHEAD):
                        _start_if(more3, k3.big(j), 1)
                if u % (NE // G) == NE // G - 1:
                    stream_scores(t1, u // (NE // G))
            macc[i] = acc
            kacc[i] = kb
            l_s[i] = tot
            inv = jnp.broadcast_to(1.0 / jnp.sum(tot, axis=1, keepdims=True), (8, DH))
            mt = acc[0:DH] * inv[0:1]
            mt_hi = mt.astype(BF)
            mhi[g * HG + i] = mt_hi
            mlo[g * HG + i] = (mt - mt_hi.astype(F32)).astype(BF)
            o8 = (acc[DH:DH + 8] + acc[DH + 8:DH + 16]) * inv
            hv[0, g, i:i + 1, :] = o8[0:1]
            hv[1, g, i:i + 1, :] = (kb[0:1] + kb[8:9]) * inv[0:1]
            col = pl.ds(pl.multiple_of(_head(g, i) * DH, DH), DH)
            o_s[:, col] = jnp.where(row8 == b, o8, o_s[:, col])
            fin.append(jnp.where(last, inv, 1.0))

        f_new = by_head(fin)
        f_old = by_head(alpha) * f_new
        for tt in range((SR - QR) // DH):
            coef[0, b, g, :, tt * DH:(tt + 1) * DH] *= f_old
        for tt in range(QR // DH):
            blk = p_s[:, (G - 1) * QR + tt * DH:(G - 1) * QR + (tt + 1) * DH]
            for st in range(G - 2, -1, -1):
                blk = jnp.where(row8 == st, p_s[:, st * QR + tt * DH:st * QR + (tt + 1) * DH], blk)
            coef[0, b, g, :, pl.ds(pl.multiple_of(rho * QR + tt * DH, DH), DH)] = blk * f_new

        pl.when(t == TPB)(lambda: wait_pieces(last_slot, R // C - NLEFT, R // C))
        return b

    def middle(b):
        add_attention(b, NG - 1)
        y1, r1 = _ln_fwd(h1_s[...])
        y2, r2 = _ln_fwd(y1)
        u = _dot(y2.astype(BF), _flat(w1_v[...]), NN) + b1_v[...].astype(F32).reshape(1, F)
        c0 = (2.0 / jnp.pi) ** 0.5
        th = jnp.tanh(c0 * (u + 0.044715 * (u * u * u)))
        dgelu = 0.5 * (1.0 + th) + 0.5 * u * (1.0 - th * th) * (c0 * (1.0 + 3 * 0.044715 * (u * u)))
        du = jnp.concatenate([dhid_s[j] for j in range(W2_SHAPE[0])], axis=1) * dgelu
        dy2 = _dot(du.astype(BF), _flat(w1_v[...]), NT)
        dh_s[...] = _rows8(g_v[...]) + _ln_bwd(_ln_bwd(dy2, y2, r2), y1, r1)
        y2_s[...] = y2
        du_s[...] = du
        hid_s[...] = 0.5 * u * (1.0 + th)

    eye = (lax.broadcasted_iota(jnp.int32, (DH, DH), 0) == lax.broadcasted_iota(jnp.int32, (DH, DH), 1))

    def fill_slot(kind, b, g, n):
        j = b * SPB + (2 * g + kind) * NN_ + n
        slot = j % NS
        drained = both(j >= SPB, j < SPB + NS - NDEF)
        pl.when(both(j >= NS, jnp.logical_not(drained)))(lambda: wait_slot(slot))

        for i in range(HG):
            w = jnp.broadcast_to(vec[kind, b, g, i:i + 1, :], (DH, DH)).astype(BF)
            tiles = []
            for z in range(SPH):
                for tt in range(R // DH):
                    r = pl.multiple_of(n * R + tt * DH, DH)
                    cf = coef[kind, b, g, pl.ds(i * SPH + z, 1), pl.ds(r, DH)]
                    tiles.append(jnp.where(eye, cf, 0.0).astype(BF))
            res = _dot(jnp.concatenate(tiles, axis=0), w, NN).astype(BF)
            for z in range(SPH):
                stage[slot, i * SPH + z] = res[z * R:(z + 1) * R]
        return j, slot

    def bwd_stream(b, g, st):
        i = st // SPH
        h = g * HG + i
        col = pl.ds(pl.multiple_of(_head(g, i) * DH, DH), DH)
        do_row = vec[0, b, g, pl.ds(i, 1), :]
        dsum = jnp.sum(do_row * hv[0, g, pl.ds(i, 1), :], axis=1, keepdims=True)
        do8 = jnp.broadcast_to(do_row, (8, DH)).astype(BF)
        dq = _dot(do8, mhi[h], NT) + _dot(do8, mlo[h], NT)
        dq = (dq - dsum * hv[1, g, pl.ds(i, 1), :]) * SCALE
        dq_s[:, col] = jnp.where(row8 == b, dq, dq_s[:, col])
        row = pl.ds(st, 1)
        for rho in range(TPG):
            dp = _dot(do8, vbuf[(b * TPB + g * TPG + rho) % NV, st], NT)
            cols = slice(rho * QR, (rho + 1) * QR)
            coef[1, b, g, row, cols] = coef[0, b, g, row, cols] * ((dp[0:1] - dsum) * SCALE)

    def group(g, b):
        do_g = _dot(dh_s[...].astype(BF), wo_group(g), NT).astype(BF).astype(F32)
        row = lax.broadcasted_iota(jnp.int32, do_g.shape, 0)
        do_b = jnp.sum(jnp.where(row == b, do_g, 0.0), axis=0, keepdims=True)
        for i in range(HG):
            vec[0, b, g, i:i + 1, :] = do_b[:, i * DH:(i + 1) * DH]

        def dv_step(n, c):
            _, slot = fill_slot(0, b, g, n)
            issue_step(dv_hbm, b, g, n, slot)
            bwd_stream(b, g, n)
            return c

        def dk_step(n, c):
            j, slot = fill_slot(1, b, g, n)
            pl.when(jnp.logical_or(j < SPB - NDEF, j >= SPB))(lambda: issue_step(dk_hbm, b, g, n, slot))
            return c

        lax.fori_loop(0, NN_, dv_step, 0)
        lax.fori_loop(0, NN_, dk_step, 0)
        return b

    def batch(b, carry):
        lax.fori_loop(0, TPB, fwd_tile, b)

        @pl.when(b == 0)
        def _():
            v_load(TPB).fine(NBL - 1).start()
            k_early = k_load(TPB + 2)
            for j in range(NBL):
                if j >= AHEAD:
                    k_early.big(j).start(priority=1)
                k_early.fine(j).start(priority=1)

        middle(b)
        lax.fori_loop(0, NG, group, b)
        return carry

    lax.fori_loop(0, B, batch, 0)

    g8 = _rows8(g_v[...])
    dh = dh_s[...]
    outs = []

    def put(src, dst, i):
        cp = misc(src, dst, i)
        cp.start()
        outs.append(cp)

    def start_all(blocks):
        def body(j, c):
            blocks.big(j).start()
            return c
        lax.fori_loop(0, blocks.n, body, 0)

    dwq_w = _Blocks(wq_v, dwq_hbm, msem.at[4], None, (8, 8, 1024), 1, 0)
    dwo_w = _Blocks(wo_v, dwo_hbm, msem.at[5], None, (8, 16, D), 1, 0)
    dw1_w = _Blocks(w1_v, dw1_hbm, msem.at[6], None, (4, 8, F // 2), 1, 0)
    dw2_w = _Blocks(w2_v, dw2_hbm, msem.at[7], None, (4, 16, D), 1, 0)

    out8 = h1_s[...] + _dot(hid_s[...].astype(BF), _flat(w2_v[...]), NN) + b2_v[...].astype(F32).reshape(1, D)
    out_v[...] = out8[0:B].astype(BF)
    put(out_v, out_hbm, 0)
    db1_v[...] = jnp.sum(du_s[...], axis=0).astype(BF)
    db2_v[...] = jnp.sum(g8, axis=0).astype(BF)
    put(db1_v, db1_hbm, 2)
    put(db2_v, db2_hbm, 3)

    def dwo_group(g, c):
        wo_v[g] = _dot(o_s[:, group_cols(g)].astype(BF), dh_s[...].astype(BF), TN).astype(BF)
        return c

    lax.fori_loop(0, NG, dwo_group, 0)
    start_all(dwo_w)

    w1_v[...] = _dot(y2_s[...].astype(BF), du_s[...].astype(BF), TN).astype(BF).reshape(W1_SHAPE)
    w2_v[...] = _dot(hid_s[...].astype(BF), g8.astype(BF), TN).astype(BF).reshape(W2_SHAPE)

    def mlp_blocks(j, c):
        dw1_w.big(j).start()
        _start_if(j < dw2_w.n, dw2_w.big(jnp.minimum(j, dw2_w.n - 1)), 0)
        return c

    lax.fori_loop(0, dw1_w.n, mlp_blocks, 0)

    xn, r0 = _ln_fwd(_rows8(x_v[...]))

    def dwq_group(g, dxn):
        cols = group_cols(g)
        dq_g = dq_s[:, cols].astype(BF)
        dxn = dxn + _dot(dq_g, _flat(wq_v[:, :, cols]), NT)
        wq_v[:, :, cols] = _dot(xn.astype(BF), dq_g, TN).astype(BF).reshape(WQ_SHAPE[0], WQ_SHAPE[1], HG * DH)
        return dxn

    dxn = lax.fori_loop(0, NG, dwq_group, jnp.zeros((8, D), F32))
    dx_v[...] = (dh + _ln_bwd(dxn, xn, r0))[0:B].astype(BF)
    put(dx_v, dx_hbm, 1)
    start_all(dwq_w)

    for slot in range(NS):
        wait_slot(slot)
    for cp in outs:
        cp.wait()
    for blocks in (dwo_w, dw1_w, dw2_w, dwq_w):
        blocks.wait_big(0, blocks.n)


@jax.jit
def pallas_sequential_preLN__mha_block_cached__mixer_channel_mlp__decode_kernel(
    A_x: jax.Array,
    A_k_cache: jax.Array,
    A_v_cache: jax.Array,
    A_wq: jax.Array,
    A_wo: jax.Array,
    B_x: jax.Array,
    B_w1: jax.Array,
    B_b1: jax.Array,
    B_w2: jax.Array,
    B_b2: jax.Array,
    grad_out: jax.Array,
):
    del B_x
    any_spec = pl.BlockSpec(memory_space=pl.ANY)
    sds = jax.ShapeDtypeStruct
    out_shape = [
        sds((B, D), BF), sds((B, D), BF), sds(KV_SHAPE, BF), sds(KV_SHAPE, BF),
        sds(WQ_SHAPE, BF), sds(WO_SHAPE, BF),
        sds(W1_SHAPE, BF), sds((F,), BF), sds(W2_SHAPE, BF), sds((D,), BF),
    ]
    vm = pltpu.VMEM
    scratch = [
        vm((NK, G, QR, DH), BF), vm((NV, G, QR, DH), BF), vm((NS, G, R, DH), BF),
        vm(WQ_SHAPE, BF), vm(WO_SHAPE, BF), vm(W1_SHAPE, BF), vm(W2_SHAPE, BF),
        vm((B, D), BF), vm((B, D), BF), vm((F,), BF), vm((D,), BF),
        vm((2, B, NG, G, SR), F32), vm((2, B, NG, 8, DH), F32),
        vm((8, H * DH), F32), vm((2, NG, 8, DH), F32), vm((8, H * DH), F32),
        vm((H, DH, DH), BF), vm((H, DH, DH), BF), vm((8, S), F32), vm((8, S), F32),
        vm((G, 8, DH), F32), vm((HG, 8, DH), F32), vm((HG, 8, DH), F32),
        vm((HG, DH + 16, DH), F32), vm((HG, 16, DH), F32),
        vm((8, D), F32), vm((8, D), F32), vm((8, D), F32), vm((8, F), F32), vm((8, F), F32),
        vm((W2_SHAPE[0], 8, W2_SHAPE[1]), F32),
        vm((B, D), BF), vm((B, D), BF), vm((F,), BF), vm((D,), BF),
        pltpu.SemaphoreType.DMA((2 * NK,)), pltpu.SemaphoreType.DMA((2 * NK,)),
        pltpu.SemaphoreType.DMA((NS,)), pltpu.SemaphoreType.DMA((12,)),
    ]
    options = dict(vmem_limit_bytes=120 * 1024 * 1024, disable_bounds_checks=True, disable_semaphore_checks=True)
    known = {f.name for f in dataclasses.fields(pltpu.CompilerParams)}
    res = pl.pallas_call(
        _kernel,
        in_specs=[any_spec] * 10,
        out_specs=[any_spec] * 10,
        out_shape=out_shape,
        scratch_shapes=scratch,
        compiler_params=pltpu.CompilerParams(**{k: v for k, v in options.items() if k in known}),
    )(A_x.reshape(B, D), A_k_cache.reshape(KV_SHAPE), A_v_cache.reshape(KV_SHAPE),
      A_wq.reshape(WQ_SHAPE), A_wo.reshape(WO_SHAPE), B_w1.reshape(W1_SHAPE), B_b1,
      B_w2.reshape(W2_SHAPE), B_b2, grad_out.reshape(B, D))
    out, dx, dk, dv, dwq, dwo, dw1, db1, dw2, db2 = res
    return (out.reshape(B, 1, D), dx.reshape(B, 1, D), dk.reshape(B, H, S, DH), dv.reshape(B, H, S, DH),
            dwq.reshape(D, H * DH), dwo.reshape(H * DH, D), dw1.reshape(D, F), db1, dw2.reshape(F, D), db2)
```

```python
import dataclasses

import jax
import jax.numpy as jnp
from jax import lax
import jax.experimental.pallas as pl
import jax.experimental.pallas.tpu as pltpu

BF = jnp.bfloat16
F32 = jnp.float32

B, H, S, DH, D, F = 2, 32, 8192, 128, 512, 1792
SCALE = DH ** -0.5
EPS = 1e-5

G = 8
SPH = 2
HG = G // SPH
SR = S // SPH
NG = H // HG
SHIFT = 1
GA = SHIFT * SPH
GB = G - GA
KV_SHAPE = (B, H * SPH, SR, DH)

QR = S // G
TPG = SR // QR
TPB = NG * TPG
T = B * TPB
NK = 3
NV = TPB + 1
BL = 64
FR = 8
BO = 8
NBL = QR // BL
LAG = 3
AHEAD = 4
MSUB = 512
NE = S // MSUB
CPS = QR // MSUB
FSKIP = (0, 3, 7, 11)
NPRE = 2
WOTICK = 6
assert NE == NBL and len(FSKIP) >= 1 + NPRE

R = 512
C = 64
CO = -24
NN_ = SR // R
SPB = 2 * NG * NN_
NS = 12
NLEFT = 1
NDEF = 8
CUTS = [0] + [c * C + CO for c in range(1, R // C)] + [R]
PIECES = [(lo, hi - lo) for lo, hi in zip(CUTS[:-1], CUTS[1:])]
assert NDEF <= NN_ and NN_ == G

WQ_SHAPE = (8, D // 8, H * DH)
WO_SHAPE = (NG, HG * DH, D)
W1_SHAPE = (4, D // 4, F)
W2_SHAPE = (4, F // 4, D)

NT = (((1,), (1,)), ((), ()))
NN = (((1,), (0,)), ((), ()))
TN = (((0,), (0,)), ((), ()))


def _dot(a, b, dims):
    return lax.dot_general(a, b, dims, preferred_element_type=F32)


def _ln_fwd(x):
    m = jnp.mean(x, axis=-1, keepdims=True)
    xc = x - m
    v = jnp.mean(xc * xc, axis=-1, keepdims=True)
    rstd = lax.rsqrt(v + EPS)
    return xc * rstd, rstd


def _ln_bwd(dy, y, rstd):
    m1 = jnp.mean(dy, axis=-1, keepdims=True)
    m2 = jnp.mean(dy * y, axis=-1, keepdims=True)
    return (dy - m1 - y * m2) * rstd


def _rows8(x2):
    return jnp.concatenate([x2.astype(F32), jnp.zeros((6, x2.shape[1]), F32)], axis=0)


def _flat(w3):
    return w3.reshape(w3.shape[0] * w3.shape[1], w3.shape[2])


def _aligned(x, n):
    return x if isinstance(x, int) else pl.multiple_of(x, n)


class _Blocks:
    def __init__(self, src, dst, sem, fsem, block, axis, fine_size):
        self.src, self.dst, self.sem, self.fsem = src, dst, sem, fsem
        self.block, self.axis, self.fine_size = block, axis, fine_size
        self.big_size = block[axis] - fine_size
        self.grid = [n // m for n, m in zip(dst.shape, block)]
        self.n = self.grid[0] * self.grid[1] * self.grid[2]

    def _part(self, j, offset, size, sem):
        at, inner = [], self.n
        for ax, align in enumerate((1, 8, DH)):
            outer, inner = inner, inner // self.grid[ax]
            pos = 0
            if self.grid[ax] > 1:
                pos = j if outer == self.n else j % outer
                pos = pos if inner == 1 else pos // inner
            lo = pos * self.block[ax] + (offset if ax == self.axis else 0)
            at.append(pl.ds(_aligned(lo, align), size if ax == self.axis else self.block[ax]))
        return pltpu.make_async_copy(self.src.at[tuple(at)], self.dst.at[tuple(at)], sem)

    def big(self, j):
        return self._part(j, 0, self.big_size, self.sem)

    def fine(self, j):
        return self._part(j, self.big_size, self.fine_size, self.fsem)

    def wait_big(self, lo, hi):
        for j in range(lo, hi):
            self.big(j).wait()

    def wait_fine(self):
        for j in range(self.n):
            self.fine(j).wait()


class _ShiftedBlocks(_Blocks):
    def big(self, j):
        if j == 0:
            return self._part(0, 0, self.big_size - BO, self.sem)
        return self._part(j, -BO, self.big_size, self.sem)

    def fine(self, j):
        return self._part(j, self.big_size - BO, self.fine_size + (BO if j == self.n - 1 else 0), self.fsem)


class _Pair:
    def __init__(self, first, second):
        self.copies = (first, second)

    def start(self, priority=0):
        for cp in self.copies:
            cp.start(priority=priority)

    def wait(self):
        for cp in self.copies:
            cp.wait()


class _BlockPairs(_Blocks):
    def __init__(self, first, second):
        self.parts, self.n = (first, second), first.n

    def big(self, j):
        return _Pair(*[p.big(j) for p in self.parts])

    def fine(self, j):
        return _Pair(*[p.fine(j) for p in self.parts])


def _head(g, i):
    return (g * HG + i + H - SHIFT) % H


def _segments(g):
    s0 = g * G - SHIFT * SPH
    return ((pl.ds((s0 + H * SPH) % (H * SPH), GA), pl.ds(0, GA)), (pl.ds(s0 + GA, GB), pl.ds(GA, GB)))


def _start_if(cond, copy, priority):
    pl.when(cond)(lambda: copy.start(priority=priority))


def _kernel(x_hbm, k_hbm, v_hbm, wq_hbm, wo_hbm, w1_hbm, b1_hbm, w2_hbm, b2_hbm, g_hbm,
            out_hbm, dx_hbm, dk_hbm, dv_hbm, dwq_hbm, dwo_hbm, dw1_hbm, db1_hbm, dw2_hbm, db2_hbm,
            kbuf, vbuf, stage, wq_v, wo_v, w1_v, w2_v, x_v, g_v, b1_v, b2_v,
            coef, vec, o_s, hv, dq_s, mhi, mlo, s_s, p_s, mx_s, m_s, l_s, macc, kacc,
            h1_s, dh_s, y2_s, du_s, hid_s, dhid_s,
            out_v, dx_v, db1_v, db2_v,
            ksem, vsem, wsem, msem):
    both = jnp.logical_and
    row8 = lax.broadcasted_iota(jnp.int32, (8, DH), 0)

    def tile_load(hbm, buf, nslot, sem, t, kind):
        rows = pl.ds(_aligned((t % TPG) * QR, QR), QR)
        return _BlockPairs(*[
            kind(hbm.at[t // TPB, far, rows], buf.at[t % nslot, near],
                 sem.at[t % NK], sem.at[NK + t % NK], (near.size, BL, DH), 1, FR)
            for far, near in _segments((t % TPB) // TPG)])

    def k_load(t, kind=_ShiftedBlocks):
        return tile_load(k_hbm, kbuf, NK, ksem, t, kind)

    def v_load(t, kind=_ShiftedBlocks):
        return tile_load(v_hbm, vbuf, NV, vsem, t, kind)

    def misc(src, dst, i):
        return pltpu.make_async_copy(src, dst, msem.at[i])

    def issue_step(dst, b, g, n, slot):
        def issue(segments):
            for lo, size in PIECES:
                rows = pl.ds(pl.multiple_of(n * R + lo, 8), size)
                for far, near in segments:
                    pltpu.make_async_copy(
                        stage.at[slot, near, pl.ds(lo, size)], dst.at[b, far, rows], wsem.at[slot]).start()

        if isinstance(g, int) and g > 0:
            issue([(pl.ds(g * G - SHIFT * SPH, G), pl.ds(0, G))])
        else:
            pl.when(g == 0)(lambda: issue(_segments(0)))
            pl.when(g > 0)(lambda: issue([(pl.ds(jnp.maximum(g * G - SHIFT * SPH, 0), G), pl.ds(0, G))]))

    def wait_slot(slot):
        pltpu.make_async_copy(stage.at[slot], stage.at[slot], wsem.at[slot]).wait()

    def wait_pieces(slot, lo, hi):
        for row, size in PIECES[lo:hi]:
            piece = stage.at[slot, :, pl.ds(row, size)]
            pltpu.make_async_copy(piece, piece, wsem.at[slot]).wait()

    def wo_group(g):
        cut = (HG - SHIFT) * DH
        return jnp.concatenate([wo_v[(g + NG - 1) % NG, cut:, :], wo_v[g, :cut, :]], axis=0)

    def group_cols(g):
        return pl.ds(_aligned(g * (HG * DH), HG * DH), HG * DH)

    def chunk_scores(t, st, c):
        q_row = vec[1, t // TPB, (t % TPB) // TPG, pl.ds(st // SPH, 1), :]
        q8 = jnp.broadcast_to(q_row, (8, DH)).astype(BF)
        sc = _dot(q8, kbuf[t % NK, st, c * MSUB:(c + 1) * MSUB], NT)
        s_s[:, pl.ds(_aligned(st * QR + c * MSUB, MSUB), MSUB)] = sc
        mx = sc[:, 0:DH]
        for tt in range(1, MSUB // DH):
            mx = jnp.maximum(mx, sc[:, tt * DH:(tt + 1) * DH])
        mx_s[st * CPS + c] = mx

    def add_attention(b, g):
        o_g = jnp.concatenate([jnp.where(row8 == b, hv[0, g, i:i + 1, :], 0.0) for i in range(HG)], axis=1)
        h1_s[...] += _dot(o_g.astype(BF), wo_group(g), NN)

    in_small = [misc(x_hbm, x_v, 0), misc(g_hbm, g_v, 1), misc(b1_hbm, b1_v, 2), misc(b2_hbm, b2_v, 3)]
    wq_l = _Blocks(wq_hbm, wq_v, msem.at[4], msem.at[8], (8, 8, 1024), 2, DH)
    wo_l = _Blocks(wo_hbm, wo_v, msem.at[5], msem.at[9], (4, 32, D), 1, 8)
    w1_l = _Blocks(w1_hbm, w1_v, msem.at[6], msem.at[10], (4, 8, F), 2, 2 * DH)
    w2_l = _Blocks(w2_hbm, w2_v, msem.at[7], msem.at[11], (4, 32, D), 1, 8)
    lag, depth = LAG + 1, LAG + 1 + AHEAD

    def paced(cur, nxt, count, work=None):
        def body(f, c):
            cur.big(f).wait()
            jf, jb = f + lag, f + depth
            _start_if(jf < cur.n, cur.fine(jnp.minimum(jf, cur.n - 1)), 0)
            _start_if(jf >= cur.n, nxt.fine(jnp.maximum(jf - cur.n, 0)), 0)
            _start_if(jb < cur.n, cur.big(jnp.minimum(jb, cur.n - 1)), 1)
            _start_if(jb >= cur.n, nxt.big(jnp.maximum(jb - cur.n, 0)), 1)
            if work is not None:
                pl.when(f % 2 == 0)(lambda: work(f // 2))
            return c
        lax.fori_loop(0, count, body, 0)

    for j in range(depth):
        wq_l.big(j).start(priority=1)
        if j == 0:
            for cp in in_small:
                cp.start()
        if j < lag:
            wq_l.fine(j).start()

    o_s[...] = jnp.zeros(o_s.shape, F32)
    dq_s[...] = jnp.zeros(dq_s.shape, F32)

    for cp in in_small:
        cp.wait()
    x8 = _rows8(x_v[...])
    h1_s[...] = x8
    y2_s[...] = _ln_fwd(x8)[0]

    def clear_probs(j):
        coef[0, j // NG, j % NG] = jnp.zeros((G, SR), F32)

    def q_group(g):
        q_g = _dot(y2_s[...].astype(BF), _flat(wq_v[:, :, group_cols(g)]), NN).astype(BF).astype(F32)
        for bb in range(B):
            for i in range(HG):
                gg, ii = (g, i + SHIFT) if i + SHIFT < HG else ((g + 1) % NG, i + SHIFT - HG)
                vec[1, bb, gg, ii:ii + 1, :] = q_g[bb:bb + 1, i * DH:(i + 1) * DH]

    def first_scores(st):
        for c in range(CPS):
            chunk_scores(0, st, c)

    def dhid_part(j):
        @pl.when(j < W2_SHAPE[0])
        def _():
            jj = jnp.minimum(j, W2_SHAPE[0] - 1)
            dhid_s[jj] = _dot(_rows8(g_v[...]).astype(BF), w2_v[jj], NT)

    k0_l, k1_l, v0_l = k_load(0, _Blocks), k_load(1, _Blocks), v_load(0, _Blocks)
    assert wq_l.n == 2 * B * NG and NBL == 2 * NG and w1_l.n == 2 * G
    paced(wq_l, k0_l, wq_l.n, clear_probs)
    wq_l.wait_fine()
    paced(k0_l, w2_l, NBL, q_group)
    k0_l.wait_fine()
    paced(w2_l, w1_l, w2_l.n)
    w2_l.wait_fine()
    paced(w1_l, wo_l, w1_l.n, first_scores)
    paced(wo_l, k1_l, wo_l.n, dhid_part)
    w1_l.wait_fine()
    paced(k1_l, v0_l, NBL)
    wo_l.wait_fine()
    k1_l.wait_fine()
    for f in range(NBL - lag):
        v0_l.big(f).wait()
        v0_l.fine(f + lag).start()
        (v0_l.big(f + depth) if f + depth < NBL else k_load(2).big(f + depth - NBL)).start(priority=1)

    def by_head(vals):
        res = vals[HG - 1]
        for i in range(HG - 2, -1, -1):
            res = jnp.where(row8 < (i + 1) * SPH, vals[i], res)
        return res

    def fwd_tile(tb, b):
        t = b * TPB + tb
        g, rho = tb // TPG, tb % TPG
        first, last = rho == 0, rho == TPG - 1
        ks, vs = t % NK, t % NV
        more1, more2, more3 = t + 1 < T, t + 2 < T, t + 3 < T
        tail = t == T - 2
        go2 = both(more2, t != TPB)
        t1 = jnp.minimum(t + 1, T - 1)
        v0, v1, v_end = v_load(t), v_load(t1), v_load(T - 1)
        k1, k2, k3 = k_load(t1), k_load(jnp.minimum(t + 2, T - 1)), k_load(jnp.minimum(t + 3, T - 1))
        last_slot = (SPB - NDEF - 1) % NS

        def starts(f):
            if f == 0:
                _start_if(both(more1, tb > 0), v0.fine(NBL - 1), 0)
            else:
                _start_if(go2, k2.fine(f - 1), 0)
                _start_if(tail, v_end.fine(f - 1), 0)
            if f + AHEAD < NBL:
                _start_if(go2, k2.big(f + AHEAD), 1)
                _start_if(tail, v_end.big(f + AHEAD), 1)
            elif f < NBL:
                _start_if(go2, v1.big(f + AHEAD - NBL), 1)

        pl.when(both(more1, t > 0))(lambda: v0.wait_big(0, NBL - lag - NPRE))
        for z in range(NPRE):
            pl.when(both(more1, t > 0))(v0.big(NBL - lag - NPRE + z).wait)
            _start_if(both(more1, tb > 0), v0.fine(NBL - 1 - NPRE + z), 0)
        pl.when(more1)(v0.big(NBL - lag).wait)
        starts(0)

        alpha = []
        for i in range(HG):
            mx = mx_s[i * NE // HG]
            for u in range(i * NE // HG + 1, (i + 1) * NE // HG):
                mx = jnp.maximum(mx, mx_s[u])
            m_blk = jnp.broadcast_to(jnp.max(mx, axis=1, keepdims=True), (8, DH))
            m_old = jnp.where(first, m_blk, m_s[i])
            m_new = jnp.maximum(m_old, m_blk)
            m_s[i] = m_new
            alpha.append(jnp.exp((m_old - m_new) * SCALE))

        for f in range(NBL):
            cols = slice(f * MSUB, (f + 1) * MSUB)
            m = jnp.concatenate([m_s[f // (NE // HG)]] * (MSUB // DH), axis=1)
            p_s[:, cols] = jnp.exp((s_s[:, cols] - m) * SCALE)
            if f == WOTICK:
                pl.when(both(first, g > 0))(lambda: add_attention(b, jnp.maximum(g - 1, 0)))
            if f < LAG:
                v0.big(NBL - LAG + f).wait()
            else:
                pl.when(more2)(k2.big(f - LAG).wait)
                pl.when(tail)(v_end.big(f - LAG).wait)
            starts(f + 1)

        pl.when(t > 0)(v0.wait_fine)
        pl.when(t == 0)(v0_l.wait_fine)

        @pl.when(both(more1, t > 0))
        def _():
            k1.wait_big(NBL - LAG, NBL)
            k1.wait_fine()

        @pl.when(tail)
        def _():
            def issue_deferred(n, c):
                issue_step(dk_hbm, 0, NG - 1, n, (SPB - NN_ + n) % NS)
                return c
            lax.fori_loop(NN_ - NDEF, NN_, issue_deferred, 0)

        @pl.when(t == TPB)
        def _():
            for j in range(SPB - NS, SPB - NDEF - 1):
                wait_slot(j % NS)
            wait_pieces(last_slot, 0, R // C - NLEFT)
            for j in range(AHEAD):
                v_load(TPB + 1).big(j).start(priority=1)

        fin = []
        for i in range(HG):
            acc = jnp.where(first, 0.0, macc[i] * alpha[i][0:1])
            kb = jnp.where(first, 0.0, kacc[i] * alpha[i][0:1])
            tot = jnp.where(first, 0.0, l_s[i] * alpha[i])
            for u in range(i * NE // HG, (i + 1) * NE // HG):
                if u not in FSKIP:
                    _start_if(more2, v1.fine(u - sum(x < u for x in FSKIP)), 0)
                if u + AHEAD < NBL:
                    _start_if(more2, v1.big(u + AHEAD), 1)
                else:
                    _start_if(t == T - 3, v_end.big(u + AHEAD - NBL), 1)
                r = u * MSUB
                st, r0 = r // QR, r % QR
                kc = kbuf[ks, st, r0:r0 + MSUB, :]
                p8 = p_s[:, r:r + MSUB]
                for tt in range(MSUB // DH):
                    tot = tot + p8[:, tt * DH:(tt + 1) * DH]
                p_hi = p8.astype(BF).astype(F32)
                p16 = jnp.concatenate([p_hi, p8 - p_hi], axis=0)
                a = kc.astype(F32).T * p_s[0:1, r:r + MSUB]
                lhs = jnp.concatenate([a, p16], axis=0).astype(BF)
                acc = acc + _dot(lhs, vbuf[vs, st, r0:r0 + MSUB, :], NN)
                kb = kb + _dot(p16.astype(BF), kc, NN)
                if u == NE - 1:
                    for j in range(NE - len(FSKIP), NBL - 1 - NPRE):
                        _start_if(more2, v1.fine(j), 0)
                    for j in range(AHEAD):
                        _start_if(more3, k3.big(j), 1)
                chunk_scores(t1, u // CPS, u % CPS)
            macc[i] = acc
            kacc[i] = kb
            l_s[i] = tot
            inv = jnp.broadcast_to(1.0 / jnp.sum(tot, axis=1, keepdims=True), (8, DH))
            mt = acc[0:DH] * inv[0:1]
            mt_hi = mt.astype(BF)
            mhi[g * HG + i] = mt_hi
            mlo[g * HG + i] = (mt - mt_hi.astype(F32)).astype(BF)
            o8 = (acc[DH:DH + 8] + acc[DH + 8:DH + 16]) * inv
            hv[0, g, i:i + 1, :] = o8[0:1]
            hv[1, g, i:i + 1, :] = (kb[0:1] + kb[8:9]) * inv[0:1]
            col = pl.ds(pl.multiple_of(_head(g, i) * DH, DH), DH)
            o_s[:, col] = jnp.where(row8 == b, o8, o_s[:, col])
            fin.append(jnp.where(last, inv, 1.0))

        f_new = by_head(fin)
        f_old = by_head(alpha) * f_new
        for tt in range((SR - QR) // DH):
            coef[0, b, g, :, tt * DH:(tt + 1) * DH] *= f_old
        for tt in range(QR // DH):
            blk = p_s[:, (G - 1) * QR + tt * DH:(G - 1) * QR + (tt + 1) * DH]
            for st in range(G - 2, -1, -1):
                blk = jnp.where(row8 == st, p_s[:, st * QR + tt * DH:st * QR + (tt + 1) * DH], blk)
            coef[0, b, g, :, pl.ds(pl.multiple_of(rho * QR + tt * DH, DH), DH)] = blk * f_new

        pl.when(t == TPB)(lambda: wait_pieces(last_slot, R // C - NLEFT, R // C))
        return b

    def middle(b):
        add_attention(b, NG - 1)
        y1, r1 = _ln_fwd(h1_s[...])
        y2, r2 = _ln_fwd(y1)
        u = _dot(y2.astype(BF), _flat(w1_v[...]), NN) + b1_v[...].astype(F32).reshape(1, F)
        c0 = (2.0 / jnp.pi) ** 0.5
        th = jnp.tanh(c0 * (u + 0.044715 * (u * u * u)))
        dgelu = 0.5 * (1.0 + th) + 0.5 * u * (1.0 - th * th) * (c0 * (1.0 + 3 * 0.044715 * (u * u)))
        du = jnp.concatenate([dhid_s[j] for j in range(W2_SHAPE[0])], axis=1) * dgelu
        dy2 = _dot(du.astype(BF), _flat(w1_v[...]), NT)
        dh_s[...] = _rows8(g_v[...]) + _ln_bwd(_ln_bwd(dy2, y2, r2), y1, r1)
        y2_s[...] = y2
        du_s[...] = du
        hid_s[...] = 0.5 * u * (1.0 + th)

    eye = (lax.broadcasted_iota(jnp.int32, (DH, DH), 0) == lax.broadcasted_iota(jnp.int32, (DH, DH), 1))

    def fill_slot(kind, b, g, n):
        j = b * SPB + (2 * g + kind) * NN_ + n
        slot = j % NS
        drained = both(j >= SPB, j < SPB + NS - NDEF)
        pl.when(both(j >= NS, jnp.logical_not(drained)))(lambda: wait_slot(slot))

        for i in range(HG):
            w = jnp.broadcast_to(vec[kind, b, g, i:i + 1, :], (DH, DH)).astype(BF)
            tiles = []
            for z in range(SPH):
                for tt in range(R // DH):
                    r = pl.multiple_of(n * R + tt * DH, DH)
                    cf = coef[kind, b, g, pl.ds(i * SPH + z, 1), pl.ds(r, DH)]
                    tiles.append(jnp.where(eye, cf, 0.0).astype(BF))
            res = _dot(jnp.concatenate(tiles, axis=0), w, NN).astype(BF)
            for z in range(SPH):
                stage[slot, i * SPH + z] = res[z * R:(z + 1) * R]
        return j, slot

    def bwd_stream(b, g, st):
        i = st // SPH
        h = g * HG + i
        col = pl.ds(pl.multiple_of(_head(g, i) * DH, DH), DH)
        do_row = vec[0, b, g, pl.ds(i, 1), :]
        dsum = jnp.sum(do_row * hv[0, g, pl.ds(i, 1), :], axis=1, keepdims=True)
        do8 = jnp.broadcast_to(do_row, (8, DH)).astype(BF)
        dq = _dot(do8, mhi[h], NT) + _dot(do8, mlo[h], NT)
        dq = (dq - dsum * hv[1, g, pl.ds(i, 1), :]) * SCALE
        dq_s[:, col] = jnp.where(row8 == b, dq, dq_s[:, col])
        row = pl.ds(st, 1)
        for rho in range(TPG):
            dp = _dot(do8, vbuf[(b * TPB + g * TPG + rho) % NV, st], NT)
            cols = slice(rho * QR, (rho + 1) * QR)
            coef[1, b, g, row, cols] = coef[0, b, g, row, cols] * ((dp[0:1] - dsum) * SCALE)

    def group(g, b):
        do_g = _dot(dh_s[...].astype(BF), wo_group(g), NT).astype(BF).astype(F32)
        row = lax.broadcasted_iota(jnp.int32, do_g.shape, 0)
        do_b = jnp.sum(jnp.where(row == b, do_g, 0.0), axis=0, keepdims=True)
        for i in range(HG):
            vec[0, b, g, i:i + 1, :] = do_b[:, i * DH:(i + 1) * DH]

        def dv_step(n, c):
            _, slot = fill_slot(0, b, g, n)
            issue_step(dv_hbm, b, g, n, slot)
            bwd_stream(b, g, n)
            return c

        def dk_step(n, c):
            j, slot = fill_slot(1, b, g, n)
            pl.when(jnp.logical_or(j < SPB - NDEF, j >= SPB))(lambda: issue_step(dk_hbm, b, g, n, slot))
            return c

        lax.fori_loop(0, NN_, dv_step, 0)
        lax.fori_loop(0, NN_, dk_step, 0)
        return b

    def batch(b, carry):
        lax.fori_loop(0, TPB, fwd_tile, b)

        @pl.when(b == 0)
        def _():
            for j in range(NBL - 1 - NPRE, NBL):
                v_load(TPB).fine(j).start()
            k_early = k_load(TPB + 2)
            for j in range(NBL):
                if j >= AHEAD:
                    k_early.big(j).start(priority=1)
                k_early.fine(j).start(priority=1)

        middle(b)
        lax.fori_loop(0, NG, group, b)
        return carry

    lax.fori_loop(0, B, batch, 0)

    g8 = _rows8(g_v[...])
    dh = dh_s[...]
    outs = []

    def put(src, dst, i):
        cp = misc(src, dst, i)
        cp.start()
        outs.append(cp)

    def start_all(blocks):
        def body(j, c):
            blocks.big(j).start()
            return c
        lax.fori_loop(0, blocks.n, body, 0)

    dwq_w = _Blocks(wq_v, dwq_hbm, msem.at[4], None, (8, 8, 1024), 1, 0)
    dwo_w = _Blocks(wo_v, dwo_hbm, msem.at[5], None, (8, 16, D), 1, 0)
    dw1_w = _Blocks(w1_v, dw1_hbm, msem.at[6], None, (4, 8, F // 2), 1, 0)
    dw2_w = _Blocks(w2_v, dw2_hbm, msem.at[7], None, (4, 16, D), 1, 0)

    out8 = h1_s[...] + _dot(hid_s[...].astype(BF), _flat(w2_v[...]), NN) + b2_v[...].astype(F32).reshape(1, D)
    out_v[...] = out8[0:B].astype(BF)
    put(out_v, out_hbm, 0)
    db1_v[...] = jnp.sum(du_s[...], axis=0).astype(BF)
    db2_v[...] = jnp.sum(g8, axis=0).astype(BF)
    put(db1_v, db1_hbm, 2)
    put(db2_v, db2_hbm, 3)

    def dwo_group(g, c):
        wo_v[g] = _dot(o_s[:, group_cols(g)].astype(BF), dh_s[...].astype(BF), TN).astype(BF)
        return c

    lax.fori_loop(0, NG, dwo_group, 0)
    start_all(dwo_w)

    w1_v[...] = _dot(y2_s[...].astype(BF), du_s[...].astype(BF), TN).astype(BF).reshape(W1_SHAPE)
    w2_v[...] = _dot(hid_s[...].astype(BF), g8.astype(BF), TN).astype(BF).reshape(W2_SHAPE)

    def mlp_blocks(j, c):
        dw1_w.big(j).start()
        _start_if(j < dw2_w.n, dw2_w.big(jnp.minimum(j, dw2_w.n - 1)), 0)
        return c

    lax.fori_loop(0, dw1_w.n, mlp_blocks, 0)

    xn, r0 = _ln_fwd(_rows8(x_v[...]))

    def dwq_group(g, dxn):
        cols = group_cols(g)
        dq_g = dq_s[:, cols].astype(BF)
        dxn = dxn + _dot(dq_g, _flat(wq_v[:, :, cols]), NT)
        wq_v[:, :, cols] = _dot(xn.astype(BF), dq_g, TN).astype(BF).reshape(WQ_SHAPE[0], WQ_SHAPE[1], HG * DH)
        return dxn

    dxn = lax.fori_loop(0, NG, dwq_group, jnp.zeros((8, D), F32))
    dx_v[...] = (dh + _ln_bwd(dxn, xn, r0))[0:B].astype(BF)
    put(dx_v, dx_hbm, 1)
    start_all(dwq_w)

    for slot in range(NS):
        wait_slot(slot)
    for cp in outs:
        cp.wait()
    for blocks in (dwo_w, dw1_w, dw2_w, dwq_w):
        blocks.wait_big(0, blocks.n)


@jax.jit
def pallas_sequential_preLN__mha_block_cached__mixer_channel_mlp__decode_kernel(
    A_x: jax.Array,
    A_k_cache: jax.Array,
    A_v_cache: jax.Array,
    A_wq: jax.Array,
    A_wo: jax.Array,
    B_x: jax.Array,
    B_w1: jax.Array,
    B_b1: jax.Array,
    B_w2: jax.Array,
    B_b2: jax.Array,
    grad_out: jax.Array,
):
    del B_x
    any_spec = pl.BlockSpec(memory_space=pl.ANY)
    sds = jax.ShapeDtypeStruct
    out_shape = [
        sds((B, D), BF), sds((B, D), BF), sds(KV_SHAPE, BF), sds(KV_SHAPE, BF),
        sds(WQ_SHAPE, BF), sds(WO_SHAPE, BF),
        sds(W1_SHAPE, BF), sds((F,), BF), sds(W2_SHAPE, BF), sds((D,), BF),
    ]
    vm = pltpu.VMEM
    scratch = [
        vm((NK, G, QR, DH), BF), vm((NV, G, QR, DH), BF), vm((NS, G, R, DH), BF),
        vm(WQ_SHAPE, BF), vm(WO_SHAPE, BF), vm(W1_SHAPE, BF), vm(W2_SHAPE, BF),
        vm((B, D), BF), vm((B, D), BF), vm((F,), BF), vm((D,), BF),
        vm((2, B, NG, G, SR), F32), vm((2, B, NG, 8, DH), F32),
        vm((8, H * DH), F32), vm((2, NG, 8, DH), F32), vm((8, H * DH), F32),
        vm((H, DH, DH), BF), vm((H, DH, DH), BF), vm((8, S), F32), vm((8, S), F32),
        vm((NE, 8, DH), F32), vm((HG, 8, DH), F32), vm((HG, 8, DH), F32),
        vm((HG, DH + 16, DH), F32), vm((HG, 16, DH), F32),
        vm((8, D), F32), vm((8, D), F32), vm((8, D), F32), vm((8, F), F32), vm((8, F), F32),
        vm((W2_SHAPE[0], 8, W2_SHAPE[1]), F32),
        vm((B, D), BF), vm((B, D), BF), vm((F,), BF), vm((D,), BF),
        pltpu.SemaphoreType.DMA((2 * NK,)), pltpu.SemaphoreType.DMA((2 * NK,)),
        pltpu.SemaphoreType.DMA((NS,)), pltpu.SemaphoreType.DMA((12,)),
    ]
    options = dict(vmem_limit_bytes=120 * 1024 * 1024, disable_bounds_checks=True, disable_semaphore_checks=True)
    known = {f.name for f in dataclasses.fields(pltpu.CompilerParams)}
    res = pl.pallas_call(
        _kernel,
        in_specs=[any_spec] * 10,
        out_specs=[any_spec] * 10,
        out_shape=out_shape,
        scratch_shapes=scratch,
        compiler_params=pltpu.CompilerParams(**{k: v for k, v in options.items() if k in known}),
    )(A_x.reshape(B, D), A_k_cache.reshape(KV_SHAPE), A_v_cache.reshape(KV_SHAPE),
      A_wq.reshape(WQ_SHAPE), A_wo.reshape(WO_SHAPE), B_w1.reshape(W1_SHAPE), B_b1,
      B_w2.reshape(W2_SHAPE), B_b2, grad_out.reshape(B, D))
    out, dx, dk, dv, dwq, dwo, dw1, db1, dw2, db2 = res
    return (out.reshape(B, 1, D), dx.reshape(B, 1, D), dk.reshape(B, H, S, DH), dv.reshape(B, H, S, DH),
            dwq.reshape(D, H * DH), dwo.reshape(H * DH, D), dw1.reshape(D, F), db1, dw2.reshape(F, D), db2)
```

```python
import dataclasses

import jax
import jax.numpy as jnp
from jax import lax
import jax.experimental.pallas as pl
import jax.experimental.pallas.tpu as pltpu

BF = jnp.bfloat16
F32 = jnp.float32

B, H, S, DH, D, F = 2, 32, 8192, 128, 512, 1792
SCALE = DH ** -0.5
EPS = 1e-5

G = 8
SPH = 2
HG = G // SPH
SR = S // SPH
NG = H // HG
SHIFT = 1
GA = SHIFT * SPH
GB = G - GA
KV_SHAPE = (B, H * SPH, SR, DH)

QR = S // G
TPG = SR // QR
TPB = NG * TPG
T = B * TPB
NK = 3
NV = TPB + 1
BL = 64
FR = 8
BO = 8
NBL = QR // BL
LAG = 3
AHEAD = 4
MSUB = 512
NE = S // MSUB
CPS = QR // MSUB
FSKIP = (0, 3, 7, 11)
NPRE = 2
WOTICK = 6
assert NE == NBL and len(FSKIP) >= 1 + NPRE

R = 512
C = 64
CO = -24
NN_ = SR // R
SPB = 2 * NG * NN_
NS = 12
NLEFT = 1
NDEF = NN_
CUTS = [0] + [c * C + CO for c in range(1, R // C)] + [R]
PIECES = [(lo, hi - lo) for lo, hi in zip(CUTS[:-1], CUTS[1:])]
assert NN_ == G

WQ_SHAPE = (8, D // 8, H * DH)
WO_SHAPE = (NG, HG * DH, D)
W1_SHAPE = (4, D // 4, F)
W2_SHAPE = (4, F // 4, D)

NT = (((1,), (1,)), ((), ()))
NN = (((1,), (0,)), ((), ()))
TN = (((0,), (0,)), ((), ()))


def _dot(a, b, dims):
    return lax.dot_general(a, b, dims, preferred_element_type=F32)


def _ln_fwd(x):
    m = jnp.mean(x, axis=-1, keepdims=True)
    xc = x - m
    v = jnp.mean(xc * xc, axis=-1, keepdims=True)
    rstd = lax.rsqrt(v + EPS)
    return xc * rstd, rstd


def _ln_bwd(dy, y, rstd):
    m1 = jnp.mean(dy, axis=-1, keepdims=True)
    m2 = jnp.mean(dy * y, axis=-1, keepdims=True)
    return (dy - m1 - y * m2) * rstd


def _rows8(x2):
    return jnp.concatenate([x2.astype(F32), jnp.zeros((6, x2.shape[1]), F32)], axis=0)


def _flat(w3):
    return w3.reshape(w3.shape[0] * w3.shape[1], w3.shape[2])


def _aligned(x, n):
    return x if isinstance(x, int) else pl.multiple_of(x, n)


class _Blocks:
    def __init__(self, src, dst, sem, fsem, block, axis, fine_size):
        self.src, self.dst, self.sem, self.fsem = src, dst, sem, fsem
        self.block, self.axis, self.fine_size = block, axis, fine_size
        self.big_size = block[axis] - fine_size
        self.grid = [n // m for n, m in zip(dst.shape, block)]
        self.n = self.grid[0] * self.grid[1] * self.grid[2]

    def _part(self, j, offset, size, sem):
        at, inner = [], self.n
        for ax, align in enumerate((1, 8, DH)):
            outer, inner = inner, inner // self.grid[ax]
            pos = 0
            if self.grid[ax] > 1:
                pos = j if outer == self.n else j % outer
                pos = pos if inner == 1 else pos // inner
            lo = pos * self.block[ax] + (offset if ax == self.axis else 0)
            at.append(pl.ds(_aligned(lo, align), size if ax == self.axis else self.block[ax]))
        return pltpu.make_async_copy(self.src.at[tuple(at)], self.dst.at[tuple(at)], sem)

    def big(self, j):
        return self._part(j, 0, self.big_size, self.sem)

    def fine(self, j):
        return self._part(j, self.big_size, self.fine_size, self.fsem)

    def wait_big(self, lo, hi):
        for j in range(lo, hi):
            self.big(j).wait()

    def wait_fine(self):
        for j in range(self.n):
            self.fine(j).wait()


class _ShiftedBlocks(_Blocks):
    def big(self, j):
        if j == 0:
            return self._part(0, 0, self.big_size - BO, self.sem)
        return self._part(j, -BO, self.big_size, self.sem)

    def fine(self, j):
        return self._part(j, self.big_size - BO, self.fine_size + (BO if j == self.n - 1 else 0), self.fsem)


class _Pair:
    def __init__(self, first, second):
        self.copies = (first, second)

    def start(self, priority=0):
        for cp in self.copies:
            cp.start(priority=priority)

    def wait(self):
        for cp in self.copies:
            cp.wait()


class _BlockPairs(_Blocks):
    def __init__(self, first, second):
        self.parts, self.n = (first, second), first.n

    def big(self, j):
        return _Pair(*[p.big(j) for p in self.parts])

    def fine(self, j):
        return _Pair(*[p.fine(j) for p in self.parts])


def _head(g, i):
    return (g * HG + i + H - SHIFT) % H


def _segments(g):
    s0 = g * G - SHIFT * SPH
    return ((pl.ds((s0 + H * SPH) % (H * SPH), GA), pl.ds(0, GA)), (pl.ds(s0 + GA, GB), pl.ds(GA, GB)))


def _start_if(cond, copy, priority):
    pl.when(cond)(lambda: copy.start(priority=priority))


def _kernel(x_hbm, k_hbm, v_hbm, wq_hbm, wo_hbm, w1_hbm, b1_hbm, w2_hbm, b2_hbm, g_hbm,
            out_hbm, dx_hbm, dk_hbm, dv_hbm, dwq_hbm, dwo_hbm, dw1_hbm, db1_hbm, dw2_hbm, db2_hbm,
            kbuf, vbuf, stage, wq_v, wo_v, w1_v, w2_v, x_v, g_v, b1_v, b2_v,
            coef, vec, o_s, hv, dq_s, mhi, mlo, s_s, p_s, mx_s, m_s, l_s, macc, kacc,
            h1_s, dh_s, y2_s, du_s, hid_s, dhid_s,
            out_v, dx_v, db1_v, db2_v,
            ksem, vsem, wsem, msem):
    both = jnp.logical_and
    row8 = lax.broadcasted_iota(jnp.int32, (8, DH), 0)

    def tile_load(hbm, buf, nslot, sem, t, kind):
        rows = pl.ds(_aligned((t % TPG) * QR, QR), QR)
        return _BlockPairs(*[
            kind(hbm.at[t // TPB, far, rows], buf.at[t % nslot, near],
                 sem.at[t % NK], sem.at[NK + t % NK], (near.size, BL, DH), 1, FR)
            for far, near in _segments((t % TPB) // TPG)])

    def k_load(t, kind=_ShiftedBlocks):
        return tile_load(k_hbm, kbuf, NK, ksem, t, kind)

    def v_load(t):
        return tile_load(v_hbm, vbuf, NV, vsem, t, _ShiftedBlocks)

    def misc(src, dst, i):
        return pltpu.make_async_copy(src, dst, msem.at[i])

    def step_copies(dst, b, segments, n, slot):
        return [pltpu.make_async_copy(stage.at[slot, near, pl.ds(lo, size)],
                                      dst.at[b, far, pl.ds(_aligned(n * R + lo, 8), size)], wsem.at[slot])
                for lo, size in PIECES for far, near in segments]

    def whole(g):
        s0 = g * G - SHIFT * SPH
        return [(pl.ds(s0 if isinstance(g, int) else jnp.maximum(s0, 0), G), pl.ds(0, G))]

    def issue_step(dst, b, g, n, slot):
        def issue(segments):
            for cp in step_copies(dst, b, segments, n, slot):
                cp.start()

        if isinstance(g, int) and g > 0:
            issue(whole(g))
        else:
            pl.when(g == 0)(lambda: issue(_segments(0)))
            pl.when(g > 0)(lambda: issue(whole(g)))

    def wait_slot(slot):
        pltpu.make_async_copy(stage.at[slot], stage.at[slot], wsem.at[slot]).wait()

    def wo_group(g):
        cut = (HG - SHIFT) * DH
        return jnp.concatenate([wo_v[(g + NG - 1) % NG, cut:, :], wo_v[g, :cut, :]], axis=0)

    def group_cols(g):
        return pl.ds(_aligned(g * (HG * DH), HG * DH), HG * DH)

    def chunk_scores(t, st, c):
        q_row = vec[1, t // TPB, (t % TPB) // TPG, pl.ds(st // SPH, 1), :]
        q8 = jnp.broadcast_to(q_row, (8, DH)).astype(BF)
        sc = _dot(q8, kbuf[t % NK, st, c * MSUB:(c + 1) * MSUB], NT)
        s_s[:, pl.ds(_aligned(st * QR + c * MSUB, MSUB), MSUB)] = sc
        mx = sc[:, 0:DH]
        for tt in range(1, MSUB // DH):
            mx = jnp.maximum(mx, sc[:, tt * DH:(tt + 1) * DH])
        mx_s[st * CPS + c] = mx

    def add_attention(b, g):
        o_g = jnp.concatenate([jnp.where(row8 == b, hv[0, g, i:i + 1, :], 0.0) for i in range(HG)], axis=1)
        h1_s[...] += _dot(o_g.astype(BF), wo_group(g), NN)

    in_small = [misc(x_hbm, x_v, 0), misc(g_hbm, g_v, 1), misc(b1_hbm, b1_v, 2), misc(b2_hbm, b2_v, 3)]
    wq_l = _Blocks(wq_hbm, wq_v, msem.at[4], msem.at[8], (8, 8, 1024), 2, DH)
    wo_l = _Blocks(wo_hbm, wo_v, msem.at[5], msem.at[9], (4, 32, D), 1, 8)
    w1_l = _Blocks(w1_hbm, w1_v, msem.at[6], msem.at[10], (4, 8, F), 2, 2 * DH)
    w2_l = _Blocks(w2_hbm, w2_v, msem.at[7], msem.at[11], (4, 32, D), 1, 8)
    lag, depth = LAG + 1, LAG + 1 + AHEAD

    def paced(cur, nxt, work=None):
        def body(f, c):
            cur.big(f).wait()
            jf, jb = f + lag, f + depth
            _start_if(jf < cur.n, cur.fine(jnp.minimum(jf, cur.n - 1)), 0)
            _start_if(jf >= cur.n, nxt.fine(jnp.maximum(jf - cur.n, 0)), 0)
            _start_if(jb < cur.n, cur.big(jnp.minimum(jb, cur.n - 1)), 1)
            _start_if(jb >= cur.n, nxt.big(jnp.maximum(jb - cur.n, 0)), 1)
            if work is not None:
                pl.when(f % 2 == 0)(lambda: work(f // 2))
            return c
        lax.fori_loop(0, cur.n, body, 0)

    for j in range(depth):
        wq_l.big(j).start(priority=1)
        if j == 0:
            for cp in in_small:
                cp.start()
        if j < lag:
            wq_l.fine(j).start()

    o_s[...] = jnp.zeros(o_s.shape, F32)
    dq_s[...] = jnp.zeros(dq_s.shape, F32)

    for cp in in_small:
        cp.wait()
    x8 = _rows8(x_v[...])
    h1_s[...] = x8
    y2_s[...] = _ln_fwd(x8)[0]

    def clear_probs(j):
        coef[0, j // NG, j % NG] = jnp.zeros((G, SR), F32)

    def q_group(g):
        q_g = _dot(y2_s[...].astype(BF), _flat(wq_v[:, :, group_cols(g)]), NN).astype(BF).astype(F32)
        for bb in range(B):
            for i in range(HG):
                gg, ii = (g, i + SHIFT) if i + SHIFT < HG else ((g + 1) % NG, i + SHIFT - HG)
                vec[1, bb, gg, ii:ii + 1, :] = q_g[bb:bb + 1, i * DH:(i + 1) * DH]

    def first_scores(st):
        for c in range(CPS):
            chunk_scores(0, st, c)

    def dhid_part(j):
        @pl.when(j < W2_SHAPE[0])
        def _():
            jj = jnp.minimum(j, W2_SHAPE[0] - 1)
            dhid_s[jj] = _dot(_rows8(g_v[...]).astype(BF), w2_v[jj], NT)

    k0_l, k1_l = k_load(0, _Blocks), k_load(1, _Blocks)
    assert wq_l.n == 2 * B * NG and NBL == 2 * NG and w1_l.n == 2 * G
    paced(wq_l, k0_l, clear_probs)
    wq_l.wait_fine()
    paced(k0_l, w2_l, q_group)
    k0_l.wait_fine()
    paced(w2_l, w1_l)
    w2_l.wait_fine()
    paced(w1_l, wo_l, first_scores)
    paced(wo_l, k1_l, dhid_part)
    w1_l.wait_fine()
    wo_l.wait_fine()
    tiles = (k1_l, v_load(0), k_load(2))
    for f in range(2 * NBL - lag):
        tiles[f // NBL].big(f % NBL).wait()
        tiles[(f + lag) // NBL].fine((f + lag) % NBL).start()
        tiles[(f + depth) // NBL].big((f + depth) % NBL).start(priority=1)
    k1_l.wait_fine()

    def by_head(vals):
        res = vals[HG - 1]
        for i in range(HG - 2, -1, -1):
            res = jnp.where(row8 < (i + 1) * SPH, vals[i], res)
        return res

    def fwd_tile(tb, b):
        t = b * TPB + tb
        g, rho = tb // TPG, tb % TPG
        first, last = rho == 0, rho == TPG - 1
        ks, vs = t % NK, t % NV
        more1, more2, more3 = t + 1 < T, t + 2 < T, t + 3 < T
        tail = t == T - 2
        go2 = both(more2, t != TPB)
        t1 = jnp.minimum(t + 1, T - 1)
        v0, v1, v_end = v_load(t), v_load(t1), v_load(T - 1)
        k1, k2, k3 = k_load(t1), k_load(jnp.minimum(t + 2, T - 1)), k_load(jnp.minimum(t + 3, T - 1))
        last_writes = step_copies(dv_hbm, 0, whole(NG - 1), NN_ - 1, (SPB - NDEF - 1) % NS)

        def starts(f):
            if f == 0:
                _start_if(both(more1, tb > 0), v0.fine(NBL - 1), 0)
            else:
                _start_if(go2, k2.fine(f - 1), 0)
                _start_if(tail, v_end.fine(f - 1), 0)
            if f + AHEAD < NBL:
                _start_if(go2, k2.big(f + AHEAD), 1)
                _start_if(tail, v_end.big(f + AHEAD), 1)
            elif f < NBL:
                _start_if(go2, v1.big(f + AHEAD - NBL), 1)

        pl.when(both(more1, t > 0))(lambda: v0.wait_big(0, NBL - lag - NPRE))
        for z in range(NPRE):
            pl.when(both(more1, t > 0))(v0.big(NBL - lag - NPRE + z).wait)
            _start_if(both(more1, tb > 0), v0.fine(NBL - 1 - NPRE + z), 0)
        pl.when(more1)(v0.big(NBL - lag).wait)
        starts(0)

        alpha = []
        for i in range(HG):
            mx = mx_s[i * NE // HG]
            for u in range(i * NE // HG + 1, (i + 1) * NE // HG):
                mx = jnp.maximum(mx, mx_s[u])
            m_blk = jnp.broadcast_to(jnp.max(mx, axis=1, keepdims=True), (8, DH))
            m_old = jnp.where(first, m_blk, m_s[i])
            m_new = jnp.maximum(m_old, m_blk)
            m_s[i] = m_new
            alpha.append(jnp.exp((m_old - m_new) * SCALE))

        for f in range(NBL):
            cols = slice(f * MSUB, (f + 1) * MSUB)
            m = jnp.concatenate([m_s[f // (NE // HG)]] * (MSUB // DH), axis=1)
            p_s[:, cols] = jnp.exp((s_s[:, cols] - m) * SCALE)
            if f == WOTICK:
                pl.when(both(first, g > 0))(lambda: add_attention(b, jnp.maximum(g - 1, 0)))
            if f < LAG:
                v0.big(NBL - LAG + f).wait()
            else:
                pl.when(more2)(k2.big(f - LAG).wait)
                pl.when(tail)(v_end.big(f - LAG).wait)
            starts(f + 1)

        v0.wait_fine()

        @pl.when(both(more1, t > 0))
        def _():
            k1.wait_big(NBL - LAG, NBL)
            k1.wait_fine()

        @pl.when(tail)
        def _():
            def issue_deferred(n, c):
                issue_step(dk_hbm, 0, NG - 1, n, (SPB - NN_ + n) % NS)
                return c
            lax.fori_loop(NN_ - NDEF, NN_, issue_deferred, 0)

        @pl.when(t == TPB)
        def _():
            for j in range(SPB - NS, SPB - NDEF - 1):
                wait_slot(j % NS)
            for cp in last_writes[:-NLEFT]:
                cp.wait()
            for j in range(AHEAD):
                v_load(TPB + 1).big(j).start(priority=1)

        fin = []
        for i in range(HG):
            acc = jnp.where(first, 0.0, macc[i] * alpha[i][0:1])
            kb = jnp.where(first, 0.0, kacc[i] * alpha[i][0:1])
            tot = jnp.where(first, 0.0, l_s[i] * alpha[i])
            for u in range(i * NE // HG, (i + 1) * NE // HG):
                if u not in FSKIP:
                    _start_if(more2, v1.fine(u - sum(x < u for x in FSKIP)), 0)
                if u + AHEAD < NBL:
                    _start_if(more2, v1.big(u + AHEAD), 1)
                else:
                    _start_if(t == T - 3, v_end.big(u + AHEAD - NBL), 1)
                r = u * MSUB
                st, r0 = r // QR, r % QR
                kc = kbuf[ks, st, r0:r0 + MSUB, :]
                p8 = p_s[:, r:r + MSUB]
                for tt in range(MSUB // DH):
                    tot = tot + p8[:, tt * DH:(tt + 1) * DH]
                p_hi = p8.astype(BF).astype(F32)
                p16 = jnp.concatenate([p_hi, p8 - p_hi], axis=0)
                a = kc.astype(F32).T * p_s[0:1, r:r + MSUB]
                lhs = jnp.concatenate([a, p16], axis=0).astype(BF)
                acc = acc + _dot(lhs, vbuf[vs, st, r0:r0 + MSUB, :], NN)
                kb = kb + _dot(p16.astype(BF), kc, NN)
                if u == NE - 1:
                    for j in range(NE - len(FSKIP), NBL - 1 - NPRE):
                        _start_if(more2, v1.fine(j), 0)
                    for j in range(AHEAD):
                        _start_if(more3, k3.big(j), 1)
                chunk_scores(t1, u // CPS, u % CPS)
            macc[i] = acc
            kacc[i] = kb
            l_s[i] = tot
            inv = jnp.broadcast_to(1.0 / jnp.sum(tot, axis=1, keepdims=True), (8, DH))
            mt = acc[0:DH] * inv[0:1]
            mt_hi = mt.astype(BF)
            mhi[g * HG + i] = mt_hi
            mlo[g * HG + i] = (mt - mt_hi.astype(F32)).astype(BF)
            o8 = (acc[DH:DH + 8] + acc[DH + 8:DH + 16]) * inv
            hv[0, g, i:i + 1, :] = o8[0:1]
            hv[1, g, i:i + 1, :] = (kb[0:1] + kb[8:9]) * inv[0:1]
            col = pl.ds(pl.multiple_of(_head(g, i) * DH, DH), DH)
            o_s[:, col] = jnp.where(row8 == b, o8, o_s[:, col])
            fin.append(jnp.where(last, inv, 1.0))

        f_new = by_head(fin)
        f_old = by_head(alpha) * f_new
        for tt in range((SR - QR) // DH):
            coef[0, b, g, :, tt * DH:(tt + 1) * DH] *= f_old
        for tt in range(QR // DH):
            blk = p_s[:, (G - 1) * QR + tt * DH:(G - 1) * QR + (tt + 1) * DH]
            for st in range(G - 2, -1, -1):
                blk = jnp.where(row8 == st, p_s[:, st * QR + tt * DH:st * QR + (tt + 1) * DH], blk)
            coef[0, b, g, :, pl.ds(pl.multiple_of(rho * QR + tt * DH, DH), DH)] = blk * f_new

        for cp in last_writes[-NLEFT:]:
            pl.when(t == TPB)(cp.wait)
        return b

    def middle(b):
        add_attention(b, NG - 1)
        y1, r1 = _ln_fwd(h1_s[...])
        y2, r2 = _ln_fwd(y1)
        u = _dot(y2.astype(BF), _flat(w1_v[...]), NN) + b1_v[...].astype(F32).reshape(1, F)
        c0 = (2.0 / jnp.pi) ** 0.5
        th = jnp.tanh(c0 * (u + 0.044715 * (u * u * u)))
        dgelu = 0.5 * (1.0 + th) + 0.5 * u * (1.0 - th * th) * (c0 * (1.0 + 3 * 0.044715 * (u * u)))
        du = jnp.concatenate([dhid_s[j] for j in range(W2_SHAPE[0])], axis=1) * dgelu
        dy2 = _dot(du.astype(BF), _flat(w1_v[...]), NT)
        dh_s[...] = _rows8(g_v[...]) + _ln_bwd(_ln_bwd(dy2, y2, r2), y1, r1)
        y2_s[...] = y2
        du_s[...] = du
        hid_s[...] = 0.5 * u * (1.0 + th)

    eye = (lax.broadcasted_iota(jnp.int32, (DH, DH), 0) == lax.broadcasted_iota(jnp.int32, (DH, DH), 1))

    def fill_slot(kind, b, g, n):
        j = b * SPB + (2 * g + kind) * NN_ + n
        slot = j % NS
        drained = both(j >= SPB, j < SPB + NS - NDEF)
        pl.when(both(j >= NS, jnp.logical_not(drained)))(lambda: wait_slot(slot))

        for i in range(HG):
            w = jnp.broadcast_to(vec[kind, b, g, i:i + 1, :], (DH, DH)).astype(BF)
            tiles = []
            for z in range(SPH):
                for tt in range(R // DH):
                    r = pl.multiple_of(n * R + tt * DH, DH)
                    cf = coef[kind, b, g, pl.ds(i * SPH + z, 1), pl.ds(r, DH)]
                    tiles.append(jnp.where(eye, cf, 0.0).astype(BF))
            res = _dot(jnp.concatenate(tiles, axis=0), w, NN).astype(BF)
            for z in range(SPH):
                stage[slot, i * SPH + z] = res[z * R:(z + 1) * R]
        return j, slot

    def bwd_stream(b, g, st):
        i = st // SPH
        h = g * HG + i
        col = pl.ds(pl.multiple_of(_head(g, i) * DH, DH), DH)
        do_row = vec[0, b, g, pl.ds(i, 1), :]
        dsum = jnp.sum(do_row * hv[0, g, pl.ds(i, 1), :], axis=1, keepdims=True)
        do8 = jnp.broadcast_to(do_row, (8, DH)).astype(BF)
        dq = _dot(do8, mhi[h], NT) + _dot(do8, mlo[h], NT)
        dq = (dq - dsum * hv[1, g, pl.ds(i, 1), :]) * SCALE
        dq_s[:, col] = jnp.where(row8 == b, dq, dq_s[:, col])
        row = pl.ds(st, 1)
        for rho in range(TPG):
            dp = _dot(do8, vbuf[(b * TPB + g * TPG + rho) % NV, st], NT)
            cols = slice(rho * QR, (rho + 1) * QR)
            coef[1, b, g, row, cols] = coef[0, b, g, row, cols] * ((dp[0:1] - dsum) * SCALE)

    def group(g, b):
        do_g = _dot(dh_s[...].astype(BF), wo_group(g), NT).astype(BF).astype(F32)
        row = lax.broadcasted_iota(jnp.int32, do_g.shape, 0)
        do_b = jnp.sum(jnp.where(row == b, do_g, 0.0), axis=0, keepdims=True)
        for i in range(HG):
            vec[0, b, g, i:i + 1, :] = do_b[:, i * DH:(i + 1) * DH]

        def dv_step(n, c):
            _, slot = fill_slot(0, b, g, n)
            issue_step(dv_hbm, b, g, n, slot)
            bwd_stream(b, g, n)
            return c

        def dk_step(n, c):
            j, slot = fill_slot(1, b, g, n)
            pl.when(jnp.logical_or(j < SPB - NDEF, j >= SPB))(lambda: issue_step(dk_hbm, b, g, n, slot))
            return c

        lax.fori_loop(0, NN_, dv_step, 0)
        lax.fori_loop(0, NN_, dk_step, 0)
        return b

    def batch(b, carry):
        lax.fori_loop(0, TPB, fwd_tile, b)

        @pl.when(b == 0)
        def _():
            for j in range(NBL - 1 - NPRE, NBL):
                v_load(TPB).fine(j).start()
            k_early = k_load(TPB + 2)
            for j in range(NBL):
                if j >= AHEAD:
                    k_early.big(j).start(priority=1)
                k_early.fine(j).start(priority=1)

        middle(b)
        lax.fori_loop(0, NG, group, b)
        return carry

    lax.fori_loop(0, B, batch, 0)

    g8 = _rows8(g_v[...])
    dh = dh_s[...]
    outs = []

    def put(src, dst, i):
        cp = misc(src, dst, i)
        cp.start()
        outs.append(cp)

    def start_all(blocks):
        def body(j, c):
            blocks.big(j).start()
            return c
        lax.fori_loop(0, blocks.n, body, 0)

    dwq_w = _Blocks(wq_v, dwq_hbm, msem.at[4], None, (8, 8, 1024), 1, 0)
    dwo_w = _Blocks(wo_v, dwo_hbm, msem.at[5], None, (8, 16, D), 1, 0)
    dw1_w = _Blocks(w1_v, dw1_hbm, msem.at[6], None, (4, 8, F // 2), 1, 0)
    dw2_w = _Blocks(w2_v, dw2_hbm, msem.at[7], None, (4, 16, D), 1, 0)

    out8 = h1_s[...] + _dot(hid_s[...].astype(BF), _flat(w2_v[...]), NN) + b2_v[...].astype(F32).reshape(1, D)
    out_v[...] = out8[0:B].astype(BF)
    put(out_v, out_hbm, 0)
    db1_v[...] = jnp.sum(du_s[...], axis=0).astype(BF)
    db2_v[...] = jnp.sum(g8, axis=0).astype(BF)
    put(db1_v, db1_hbm, 2)
    put(db2_v, db2_hbm, 3)

    def dwo_group(g, c):
        wo_v[g] = _dot(o_s[:, group_cols(g)].astype(BF), dh_s[...].astype(BF), TN).astype(BF)
        return c

    lax.fori_loop(0, NG, dwo_group, 0)
    start_all(dwo_w)

    xn, r0 = _ln_fwd(_rows8(x_v[...]))

    def dwq_group(g, dxn):
        cols = group_cols(g)
        dq_g = dq_s[:, cols].astype(BF)
        dxn = dxn + _dot(dq_g, _flat(wq_v[:, :, cols]), NT)
        wq_v[:, :, cols] = _dot(xn.astype(BF), dq_g, TN).astype(BF).reshape(WQ_SHAPE[0], WQ_SHAPE[1], HG * DH)
        return dxn

    dxn = lax.fori_loop(0, NG, dwq_group, jnp.zeros((8, D), F32))
    dx_v[...] = (dh + _ln_bwd(dxn, xn, r0))[0:B].astype(BF)
    put(dx_v, dx_hbm, 1)
    start_all(dwq_w)

    w1_v[...] = _dot(y2_s[...].astype(BF), du_s[...].astype(BF), TN).astype(BF).reshape(W1_SHAPE)
    w2_v[...] = _dot(hid_s[...].astype(BF), g8.astype(BF), TN).astype(BF).reshape(W2_SHAPE)

    def mlp_blocks(j, c):
        dw1_w.big(j).start()
        _start_if(j < dw2_w.n, dw2_w.big(jnp.minimum(j, dw2_w.n - 1)), 0)
        return c

    lax.fori_loop(0, dw1_w.n, mlp_blocks, 0)

    for slot in range(NS):
        wait_slot(slot)
    for cp in outs:
        cp.wait()
    for blocks in (dwo_w, dwq_w, dw2_w, dw1_w):
        blocks.wait_big(0, blocks.n)


@jax.jit
def pallas_sequential_preLN__mha_block_cached__mixer_channel_mlp__decode_kernel(
    A_x: jax.Array,
    A_k_cache: jax.Array,
    A_v_cache: jax.Array,
    A_wq: jax.Array,
    A_wo: jax.Array,
    B_x: jax.Array,
    B_w1: jax.Array,
    B_b1: jax.Array,
    B_w2: jax.Array,
    B_b2: jax.Array,
    grad_out: jax.Array,
):
    del B_x
    any_spec = pl.BlockSpec(memory_space=pl.ANY)
    sds = jax.ShapeDtypeStruct
    out_shape = [
        sds((B, D), BF), sds((B, D), BF), sds(KV_SHAPE, BF), sds(KV_SHAPE, BF),
        sds(WQ_SHAPE, BF), sds(WO_SHAPE, BF),
        sds(W1_SHAPE, BF), sds((F,), BF), sds(W2_SHAPE, BF), sds((D,), BF),
    ]
    vm = pltpu.VMEM
    scratch = [
        vm((NK, G, QR, DH), BF), vm((NV, G, QR, DH), BF), vm((NS, G, R, DH), BF),
        vm(WQ_SHAPE, BF), vm(WO_SHAPE, BF), vm(W1_SHAPE, BF), vm(W2_SHAPE, BF),
        vm((B, D), BF), vm((B, D), BF), vm((F,), BF), vm((D,), BF),
        vm((2, B, NG, G, SR), F32), vm((2, B, NG, 8, DH), F32),
        vm((8, H * DH), F32), vm((2, NG, 8, DH), F32), vm((8, H * DH), F32),
        vm((H, DH, DH), BF), vm((H, DH, DH), BF), vm((8, S), F32), vm((8, S), F32),
        vm((NE, 8, DH), F32), vm((HG, 8, DH), F32), vm((HG, 8, DH), F32),
        vm((HG, DH + 16, DH), F32), vm((HG, 16, DH), F32),
        vm((8, D), F32), vm((8, D), F32), vm((8, D), F32), vm((8, F), F32), vm((8, F), F32),
        vm((W2_SHAPE[0], 8, W2_SHAPE[1]), F32),
        vm((B, D), BF), vm((B, D), BF), vm((F,), BF), vm((D,), BF),
        pltpu.SemaphoreType.DMA((2 * NK,)), pltpu.SemaphoreType.DMA((2 * NK,)),
        pltpu.SemaphoreType.DMA((NS,)), pltpu.SemaphoreType.DMA((12,)),
    ]
    options = dict(vmem_limit_bytes=120 * 1024 * 1024, disable_bounds_checks=True, disable_semaphore_checks=True)
    known = {f.name for f in dataclasses.fields(pltpu.CompilerParams)}
    res = pl.pallas_call(
        _kernel,
        in_specs=[any_spec] * 10,
        out_specs=[any_spec] * 10,
        out_shape=out_shape,
        scratch_shapes=scratch,
        compiler_params=pltpu.CompilerParams(**{k: v for k, v in options.items() if k in known}),
    )(A_x.reshape(B, D), A_k_cache.reshape(KV_SHAPE), A_v_cache.reshape(KV_SHAPE),
      A_wq.reshape(WQ_SHAPE), A_wo.reshape(WO_SHAPE), B_w1.reshape(W1_SHAPE), B_b1,
      B_w2.reshape(W2_SHAPE), B_b2, grad_out.reshape(B, D))
    out, dx, dk, dv, dwq, dwo, dw1, db1, dw2, db2 = res
    return (out.reshape(B, 1, D), dx.reshape(B, 1, D), dk.reshape(B, H, S, DH), dv.reshape(B, H, S, DH),
            dwq.reshape(D, H * DH), dwo.reshape(H * DH, D), dw1.reshape(D, F), db1, dw2.reshape(F, D), db2)
```
